```python
import jax
import jax.numpy as jnp

def _softmax(x, axis=-1):
    return jax.nn.softmax(x, axis=axis)
def _gelu(x):
    return jax.nn.gelu(x, approximate=True)
def _silu(x):
    return jax.nn.silu(x)
def _sigmoid(x):
    return jax.nn.sigmoid(x)
def _layernorm(x, axis=-1, eps=1e-5):
    m = jnp.mean(x, axis=axis, keepdims=True)
    v = jnp.var(x, axis=axis, keepdims=True)
    return (x - m) / jnp.sqrt(v + eps)
def _scatter_add(tgt, idx, src, axis=0):
    return tgt.at[idx].add(src)
def _segment_sum(src, seg, n):
    return jax.ops.segment_sum(src, seg, n)
class _Rng:
    def __init__(self, key):
        self._k = key
    def _next(self):
        self._k, sub = jax.random.split(self._k)
        return sub
    def normal(self, shape):
        return jax.random.normal(self._next(), shape, dtype=jnp.bfloat16)
    def randint(self, lo, hi, shape):
        return jax.random.randint(self._next(), shape, lo, hi, dtype=jnp.int32)
    def uniform(self, shape, lo=0.0, hi=1.0):
        return jax.random.uniform(self._next(), shape, jnp.bfloat16, lo, hi)
    def permutation(self, n):
        return jax.random.permutation(self._next(), n)


kernel_name = 'interleave_layers__spectral_gfnet__sliding_local_dilated__prompt'

def setup_inputs():
    _rng = _Rng(jax.random.key(int.from_bytes(__import__("os").urandom(4), "little")))
    _w = (lambda a: (lambda t: t.astype(jnp.bfloat16) if jnp.issubdtype(t.dtype, jnp.floating) else t)(jnp.asarray(a)))
    def _A_setup():
        B, S, D = 1, 2048, 1024
        Df = D // 2 + 1
        return {
            "x": _w((lambda *s: _rng.normal(s) * 0.05)(B, S, D)),
            "w_r": _w((lambda *s: _rng.normal(s) * 0.05)(S, Df) * 0.02),
            "w_i": _w((lambda *s: _rng.normal(s) * 0.05)(S, Df) * 0.02),
        }
    _A_in = _A_setup()

    def _B_setup():
        B, S, D = 1, 2048, 1024
        return {
            "x": _w((lambda *s: _rng.normal(s) * 0.05)(B, S, D)),
            "wqkv": _w((lambda *s: _rng.normal(s) * 0.05)(D, 3 * D)),
            "wo": _w((lambda *s: _rng.normal(s) * 0.05)(D, D)),
        }
    _B_in = _B_setup()

    return {
        "A_x": _A_in["x"],
        "A_w_r": _A_in["w_r"],
        "A_w_i": _A_in["w_i"],
        "B_x": _B_in["x"],
        "B_wqkv": _B_in["wqkv"],
        "B_wo": _B_in["wo"],
    }

def reference(A_x, A_w_r, A_w_i, B_x, B_wqkv, B_wo):
    def _A_ref(x, w_r, w_i):
        B, S, D = x.shape
        X = (lambda x, axes=(-2,-1): jnp.fft.rfft2(x.astype(jnp.float32), axes=axes))(x, axes=(-2, -1))
        W = w_r + 1j * w_i
        X = X * W
        y = (lambda x, s, axes=(-2,-1): jnp.fft.irfft2(x, s=s, axes=axes).astype(jnp.bfloat16))(X, (S, D), axes=(-2, -1))
        return y

    def _B_ref(x, wqkv, wo):
        B, S, D = x.shape
        H = 32; Dh = D // H
        W, dil = 8, 2
        qkv = (lambda x, *d: x.transpose(*d))((x @ wqkv).reshape(B, S, 3, H, Dh), 2, 0, 3, 1, 4)
        q, k, v = qkv[0], qkv[1], qkv[2]
        scale = Dh ** -0.5
        pos = jnp.arange(S)
        off = jnp.arange(W) * dil
        idx = pos[:, None] - off[None, :]
        mask = idx >= 0
        idx_c = jnp.where(mask, idx, 0).reshape(-1)
        kg = k[:, :, idx_c, :].reshape(B, H, S, W, Dh)
        vg = v[:, :, idx_c, :].reshape(B, H, S, W, Dh)
        logits = jnp.einsum("bhsd,bhswd->bhsw", q, kg) * scale
        logits = jnp.where(mask[None, None, :, :], logits, -1e9)
        attn = _softmax(logits, axis=-1)
        o = jnp.einsum("bhsw,bhswd->bhsd", attn, vg)
        return (lambda x, *d: x.transpose(*d))(o, 0, 2, 1, 3).reshape(B, S, D) @ wo

    x = A_x
    x = x + _A_ref(_layernorm(x, axis=-1), A_w_r, A_w_i)
    x = x + _B_ref(_layernorm(x, axis=-1), B_wqkv, B_wo)
    x = x + _A_ref(_layernorm(x, axis=-1), A_w_r, A_w_i)
    x = x + _B_ref(_layernorm(x, axis=-1), B_wqkv, B_wo)
    return x
```

```python
import functools
import numpy as np
import jax
import jax.numpy as jnp
from jax.experimental import pallas as pl
from jax.experimental.pallas import tpu as pltpu

S, D = 2048, 1024
f32, bf16, u32 = jnp.float32, jnp.bfloat16, jnp.uint32
T = 256
NB = S // T
H = T // 2
PITCH = 129
WROWS = 264
R2 = float(np.sqrt(0.5))
C8, S8 = float(np.cos(np.pi / 8)), float(np.sin(np.pi / 8))
SCALE = 2.0 / (S * D)


def _seeds():
    r = np.arange(8)[:, None]
    l = np.arange(128)[None, :]
    cls, j = l >> 6, l & 63
    tiles = []
    freqs = [8 * j, 8 * j + 4] + [8 * j + np.where(cls == 0, c, 8 - c) for c in (1, 2, 3)]
    for m in freqs:
        th, st = 2 * np.pi * r * m / D, 2 * np.pi * 8 * m / D + 0 * r
        tiles += [np.cos(th), np.sin(th), np.cos(st), np.sin(st)]
    for h in range(2):
        col = 128 * h + l
        b, odd = col >> 1, (col & 1) == 1
        al, st, tw = 2 * np.pi * r * b / 128, 2 * np.pi * 8 * b / 128 + 0 * r, 2 * np.pi * b / S + 0 * r
        tiles += [np.where(odd, np.sin(al), np.cos(al)), np.where(odd, np.cos(al), -np.sin(al)),
                  np.cos(st), np.sin(st), np.cos(tw), np.sin(tw)]
    tw = 2 * np.pi * r / S + 0 * l
    tiles += [np.cos(tw), np.sin(tw)]
    return np.stack(tiles).astype(np.float32)


def _iota(shape, axis):
    return jax.lax.broadcasted_iota(jnp.int32, shape, axis)


def _pack(a, b):
    return pltpu.pack_elementwise([a, b], packed_dtype=bf16)


def _unpack(w, i):
    return pltpu.unpack_elementwise(w, index=i, packed_dtype=bf16, unpacked_dtype=f32)


def _tiles(v):
    return [v[:, 128 * a:128 * (a + 1)] for a in range(v.shape[1] // 128)]


def _tree(op, xs):
    xs = list(xs)
    while len(xs) > 1:
        xs = [op(xs[i], xs[i + 1]) if i + 1 < len(xs) else xs[i] for i in range(0, len(xs), 2)]
    return xs[0]


def _rot(c, s, cs, ss):
    return c * cs - s * ss, s * cs + c * ss


def _layernorm(xs):
    m = jnp.sum(_tree(jnp.add, xs), axis=-1, keepdims=True) * (1.0 / D)
    xc = [x - m for x in xs]
    v = jnp.sum(_tree(jnp.add, [x * x for x in xc]), axis=-1, keepdims=True) * (1.0 / D)
    inv = jax.lax.rsqrt(v + 1e-5)
    return [x * inv for x in xc]


def _radix8_fwd(z):
    e = [z[a] + z[a + 4] for a in range(4)]
    o = [z[a] - z[a + 4] for a in range(4)]
    s02, s13 = e[0] + e[2], e[1] + e[3]
    p, q = (o[1] - o[3]) * R2, (o[1] + o[3]) * R2
    return [s02 + s13, s02 - s13, o[0] + p, o[2] + q, e[0] - e[2], e[3] - e[1], o[0] - p, o[2] - q]


def _radix8_inv(t):
    t0, t4, r1, n1, r2, i2, r3, i3 = t
    a, b = t0 + t4, t0 - t4
    E = [a + r2, b - i2, a - r2, b + i2]
    u, v = r1 - r3, i3 - n1
    O = [r1 + r3, (u - v) * R2, i3 + n1, (u + v) * (-R2)]
    return [E[k] + O[k] for k in range(4)] + [E[k] - O[k] for k in range(4)]


def _dft4(x, sgn):
    (ar, ai), (br, bi), (cr, ci), (dr, di) = x
    sr, si, tr, ti = ar + cr, ai + ci, ar - cr, ai - ci
    ur, ui, vr, vi = br + dr, bi + di, br - dr, bi - di
    y1, y3 = (tr + vi, ti - vr), (tr - vi, ti + vr)
    if sgn > 0:
        y1, y3 = y3, y1
    return [(sr + ur, si + ui), y1, (sr - ur, si - ui), y3]


def _tw16(x, k, sgn):
    xr, xi = x
    k = k % 16
    if k == 0:
        return x
    if k == 4:
        return (xi, -xr) if sgn < 0 else (-xi, xr)
    if k == 2:
        return ((xr + xi) * R2, (xi - xr) * R2) if sgn < 0 else ((xr - xi) * R2, (xi + xr) * R2)
    if k == 6:
        return ((xi - xr) * R2, (xr + xi) * (-R2)) if sgn < 0 else ((xr + xi) * (-R2), (xr - xi) * R2)
    c, s = float(np.cos(np.pi * k / 8)), float(sgn * np.sin(np.pi * k / 8))
    return (xr * c - xi * s, xi * c + xr * s)


def _dft16(x, sgn):
    cols = [_dft4([x[a2 + 4 * a1] for a1 in range(4)], sgn) for a2 in range(4)]
    out = [None] * 16
    for k1 in range(4):
        y = _dft4([_tw16(cols[a2][k1], a2 * k1, sgn) for a2 in range(4)], sgn)
        for k2 in range(4):
            out[k1 + 4 * k2] = y[k2]
    return out


def _dot(a, b):
    return jnp.dot(a, b, preferred_element_type=f32)


def _dot_nt(a, b):
    return jax.lax.dot_general(a, b, (((1,), (1,)), ((), ())), preferred_element_type=f32)


def _b(w):
    return pltpu.bitcast(w, bf16)


def _w(v):
    return pltpu.bitcast(v.astype(bf16), u32)


def _strassen_lhs(top, bot):
    a11, a12 = jnp.concatenate(top[:4], axis=1), jnp.concatenate(top[4:], axis=1)
    a21, a22 = jnp.concatenate(bot[:4], axis=1), jnp.concatenate(bot[4:], axis=1)
    return [a11 + a22, a21 + a22, a11, a22, a11 + a12, a21 - a11, a12 - a22]


def _strassen_rhs(b11, b12, b21, b22):
    def comb(p, q, op):
        return _pack(op(_unpack(p, 0), _unpack(q, 0)), op(_unpack(p, 1), _unpack(q, 1)))
    return [comb(b11, b22, jnp.add), b11, comb(b12, b22, jnp.subtract), comb(b21, b11, jnp.subtract),
            b22, comb(b11, b12, jnp.add), comb(b21, b22, jnp.add)]


def _weave(never, mm, vec):
    def gate(tokens):
        def apply(v):
            if not tokens:
                return v
            t = v[0:8, 0:128]
            for tok in tokens:
                t = jnp.where(never, tok if tok.dtype == t.dtype else pltpu.bitcast(tok, t.dtype), t)
            if v.shape[1] > 128:
                t = jnp.concatenate([t, v[0:8, 128:]], axis=1)
            return jnp.concatenate([t, v[8:]], axis=0) if v.shape[0] > 8 else t
        return apply
    done, due = {}, {}
    for n in range(-1, len(mm)):
        if n >= 0:
            done[n] = mm[n](gate(due.pop(n, [])))
        for job, after, before in vec:
            if max(after, -1) == n:
                due.setdefault(before, []).append(job(gate([done[n]] if n >= 0 else []))[0:8, 0:128])


def _spread(jobs, lo, hi, window=2):
    out = []
    for k, job in enumerate(jobs):
        n = lo + (k * (hi - lo)) // len(jobs)
        out.append((job, n - 1, min(n + window, hi)))
    return out


def _cols(j, n=1):
    return pl.ds(128 * j, 128 * n)


def _kernel(x_hbm, wr_hbm, wi_hbm, wqkv_hbm, wo_hbm, seed_hbm, out_hbm,
            seed, xin, X, Vp, U, dm, G, Gi, Wf, W0, Wq, Wo, tb0, tb1, sem):
    P_ = functools.partial

    def x_copy(i):
        return pltpu.make_async_copy(x_hbm.at[pl.ds(i * T, T)], xin.at[pl.ds(i * T, T)], sem.at[i])

    def out_copy(r0, i):
        return pltpu.make_async_copy(xin.at[pl.ds(r0, T)], out_hbm.at[pl.ds(r0, T)], sem.at[i])

    sub = _iota((8, 128), 0)
    lane = _iota((8, 128), 1)

    def weave(mm, vec):
        _weave(seed[0] > 2.0, mm, vec)

    def ln_radix8(tb, g, xs):
        w = _w(jnp.concatenate(_radix8_fwd(_layernorm(xs)), axis=1))
        tb[pl.ds(8 * g, 8), :] = w
        return w

    def dft_d(r0, tb, c, gate):
        if c == 0:
            a = _dot(_b(tb[:, 0:128]), _b(gate(dm[0, 0:64, 0:128])))
            b = _dot(_b(tb[:, 128:256]), _b(dm[0, 0:64, 128:256]))
            lo = _iota((T, 128), 1) < 64
            w = _pack(jnp.where(lo, a, b), pltpu.roll(jnp.where(lo, b, a), 64, 1))
        else:
            y = _dot(_b(tb[:, 256 * c:256 * (c + 1)]), _b(gate(dm[c])))
            w = _pack(y[:, :128], y[:, 128:])
        for g in range(T // 8):
            Vp[c, pl.ds((g % 2) * 8 * PITCH + r0 // 16 + g // 2, 8, stride=PITCH), :] = w[8 * g:8 * g + 8, :]
        return w[0:8]

    def spectral(hooks, P, Z):
        def mm1(c, a0, gate):
            for a in range(a0, a0 + 4):
                v = Vp[c, pl.ds(a * PITCH, 128), :]
                y = _dot(_b(G[a]), _b(gate(v) if a == a0 else v))
                P[c, a] = y
            return y[0:8]

        def mid(c, g, gate):
            rows, rows2 = pl.ds(8 * g, 8), pl.ds(128 + 8 * g, 8)
            x = [(P[c, a, rows, :], P[c, a, rows2, :]) for a in range(16)]
            x[0] = (gate(x[0][0]), x[0][1])
            y = _dft16(x, -1)
            if c == 0:
                part = []
                for a in range(16):
                    w1 = [P[c, a, pl.ds(o + 8 * (15 - g), 8), :] for o in (0, 128)]
                    w0 = [P[c, a, pl.ds(o + 8 * ((16 - g) % 16), 8), :] for o in (0, 128)]
                    if g == 0:
                        w0 = _tw16(w0, a, -1)
                    part.append(tuple(jnp.take_along_axis(jnp.where(sub == 0, p, q), (8 - sub) & 7, axis=0)
                                      for p, q in zip(w0, w1)))
                yp = _dft16(part, -1)
            z = []
            for k1 in range(16):
                yr, yi = y[k1]
                kr = pl.ds(128 * k1 + 8 * g, 8)
                if c == 0:
                    ar, ai, br, bi = (W0[q, kr, :] for q in range(4))
                    pr, pi = yp[15 - k1]
                    z.append(((yr * ar - yi * ai) + (pr * br + pi * bi),
                              (yr * ai + yi * ar) + (pr * bi - pi * br)))
                else:
                    w = Wf[c - 1, kr, :]
                    ar, ai = _unpack(w, 0), _unpack(w, 1)
                    z.append((yr * ar - yi * ai, yr * ai + yi * ar))
            rr = _dft16(z, 1)
            for a in range(16):
                w = _pack(*rr[a])
                Z[c, a, rows, :] = w
            return w

        def mm2(c, a0, gate):
            for a in range(a0, a0 + 4):
                v = Z[c, a]
                u = _dot(_b(Gi[a]), _b(gate(v) if a == a0 else v))
                U[0, c, pl.ds(a * PITCH, 128), :] = u[:128]
                U[1, c, pl.ds(a * PITCH, 128), :] = u[128:]
            return u[0:8]

        m1 = lambda c: [P_(mm1, c, a0) for a0 in range(0, 16, 4)]
        m2 = lambda c: [P_(mm2, c, a0) for a0 in range(0, 16, 4)]
        mids = lambda c: [P_(mid, c, g) for g in range(16)]
        if hooks is None:
            weave(m1(0) + m1(1) + m1(2) + m2(0) + m1(3) + m2(1) + m2(2) + m2(3),
                  _spread(mids(0), 4, 12) + _spread(mids(1), 10, 17) + _spread(mids(2), 16, 22)
                  + _spread(mids(3), 22, 28))
        else:
            weave(m1(0) + m1(1), [])
            hooks[0]()
            weave(m1(2) + m1(3), [])
            hooks[1]()
            weave(m2(1) + m2(2), _spread(mids(1), 0, 0, 0) + _spread(mids(2), 0, 4) + _spread(mids(3), 4, 8))
            hooks[2]()
            weave(m2(3) + m2(0), _spread(mids(0), 0, 4))
            hooks[3]()

    def run_spectral(hooks):
        pl.run_scoped(P_(spectral, hooks), pltpu.VMEM((4, 16, 256, 128), f32), pltpu.VMEM((4, 16, 128, 128), u32))

    def prologue(wr, wi, wq_raw, wo_raw, wo_u, WE):
        cp_seed = pltpu.make_async_copy(seed_hbm, seed, sem.at[NB])
        cp_w = [pltpu.make_async_copy(src.at[:, pl.ds(512 * n, 512)], dst.at[:, pl.ds(512 * n, 512)],
                                      sem.at[NB + 1 + 2 * n + q])
                for n in range(4) for q, (src, dst) in enumerate(((wr_hbm, wr), (wi_hbm, wi)))]
        cp_q = [pltpu.make_async_copy(wqkv_hbm.at[:, pl.ds(D * n, D)], wq_raw.at[:, pl.ds(D * n, D)],
                                      sem.at[NB + 9 + n]) for n in range(3)]
        cp_o = pltpu.make_async_copy(wo_hbm, wo_raw, sem.at[NB + 12])
        cp_seed.start()
        for i in range(NB):
            x_copy(i).start()
        cp_seed.wait()

        lane16 = _iota((16, 128), 1)
        lo = lane16 < 64
        for n in range(5):
            c, s, cs, ss = (seed[4 * n + q] for q in range(4))
            for g in range(8):
                c2, s2 = _rot(c, s, cs, ss)
                cc, sc = jnp.concatenate([c, c2], axis=0), jnp.concatenate([s, s2], axis=0)
                rows, rows2 = pl.ds(8 * g, 8), pl.ds(64 + 8 * g, 8)
                if n == 0:
                    alt = (1 - 2 * (_iota((16, 128), 0) & 1)).astype(f32)
                    dm[0, rows, 0:128] = _w(jnp.where(lane16 == 64, alt, jnp.where(lo, cc, -sc)))
                elif n == 1:
                    dm[0, rows, 128:256] = _w(jnp.where(lo, -sc, cc))
                else:
                    sg = jnp.where(lo, 1.0, -1.0) * (-1.0 if n == 2 else 1.0)
                    dm[n - 1, rows, 0:128] = _w(cc)
                    dm[n - 1, rows, 128:256] = _w(-sc)
                    dm[n - 1, rows2, 0:128] = _w(sg * sc)
                    dm[n - 1, rows2, 128:256] = _w(sg * cc)
                if g < 7:
                    c, s = _rot(c2, s2, cs, ss)

        def gen(q, carry):
            rows = pl.ds(pl.multiple_of(q * 8, 8), 8)
            rows2 = pl.ds(pl.multiple_of(64 + q * 8, 8), 8)
            c1, s1 = float(np.cos(2 * np.pi * 8 / S)), float(np.sin(2 * np.pi * 8 / S))
            cb0, sb0 = carry[4], carry[5]
            cb1, sb1 = _rot(cb0, sb0, c1, s1)
            cb, sb = jnp.concatenate([cb0, cb1], axis=0), jnp.concatenate([sb0, sb1], axis=0)
            sg = (1 - 2 * (lane16 & 1)).astype(f32)
            new = []
            for h in range(2):
                p0, q0 = carry[2 * h], carry[2 * h + 1]
                cs, ss, ct, st = (seed[22 + 6 * h + n] for n in range(4))
                q1, p1 = _rot(q0, p0, cs, ss)
                p, q_ = jnp.concatenate([p0, p1], axis=0), jnp.concatenate([q0, q1], axis=0)
                pi, qi = p * (sg * SCALE), q_ * (-sg * SCALE)
                ct, st = jnp.concatenate([ct, ct], axis=0), jnp.concatenate([st, st], axis=0)
                for a in range(16):
                    G[a, rows, _cols(h)] = _w(p)
                    G[a, rows2, _cols(h)] = _w(q_)
                    Gi[a, rows, _cols(h)] = _w(pi)
                    Gi[a, rows2, _cols(h)] = _w(qi)
                    if a < 15:
                        q_, p = _rot(q_, p, cb, sb)
                        pi, qi = _rot(pi, qi, ct, st)
                q2, p2 = _rot(q1, p1, cs, ss)
                new += [p2, q2]
            return tuple(new) + _rot(cb1, sb1, c1, s1)
        jax.lax.fori_loop(0, 8, gen, (seed[20], seed[21], seed[26], seed[27], seed[32], seed[33]))

        def ln_x(i, g, gate):
            xs = _tiles(xin[pl.ds(i * T + 16 * g, 16), :].astype(f32))
            xs[0] = gate(xs[0])
            return ln_radix8((tb0, tb1)[i % 2], g, xs)

        for i in range(-1, NB):
            vec = []
            if i + 1 < NB:
                x_copy(i + 1).wait()
                if i + 1 == NB - 3:
                    for cp in cp_w:
                        cp.start()
                vec = [P_(ln_x, i + 1, g) for g in range(T // 16)]
            if i < 0:
                weave([], _spread(vec, 0, 0))
            else:
                weave([P_(dft_d, i * T, (tb0, tb1)[i % 2], c) for c in range(4)], _spread(vec, 0, 4))

        def filter_prep(n):
            cp_w[2 * n].wait()
            cp_w[2 * n + 1].wait()
            for t in range(4 * n, 4 * n + 4):
                we = WE.at[t % 2]
                a = pltpu.bitcast(wr[0:512, _cols(t)], u32)
                b = pltpu.bitcast(wi[0:512, _cols(t)], u32)
                we[0] = (a & 0xFFFF) | (b << 16)
                we[1] = (a >> 16) | (b & jnp.uint32(0xFFFF0000))
                for c in range(4):
                    r0, r1 = c, (8 - c) if c else 4
                    w = jnp.concatenate([we[r & 1, pl.ds(r >> 1, 64, stride=4), :] for r in (r0, r1)], axis=0).T
                    if c:
                        Wf[c - 1, pl.ds(128 * t, 128), :] = w
                    else:
                        U[0, 0, pl.ds(128 * t, 128), :] = _unpack(w, 0)
                        U[0, 1, pl.ds(128 * t, 128), :] = _unpack(w, 1)
                for q, src in enumerate((wr, wi)):
                    last = jnp.broadcast_to(src[512:513, _cols(t)].astype(f32), (128, 128))
                    U[1, q, pl.ds(128 * t, 128), :] = last.T

        def filter_pair():
            def body(g, _):
                l0 = lane == 0
                rows = pl.ds(pl.multiple_of(8 * g, 8), 8)
                r1 = pl.ds(pl.multiple_of(8 * (255 - g), 8), 8)
                r0 = pl.ds(pl.multiple_of(8 * ((256 - g) & 255), 8), 8)
                ar, ai, br, bi = (U[q >> 1, q & 1, rows, :] for q in range(4))
                cr, ci, dr, di = (
                    jnp.take_along_axis(jnp.where(sub == 0, U[q >> 1, q & 1, r0, :], U[q >> 1, q & 1, r1, :]),
                                        (8 - sub) & 7, axis=0) for q in range(4))
                W0[0, rows, :] = jnp.where(l0, ((ar + br) + (cr + dr)) * 0.125, ar)
                W0[1, rows, :] = jnp.where(l0, ((ai + bi) - (ci + di)) * 0.125, ai)
                W0[2, rows, :] = jnp.where(l0, ((ar - br) + (cr - dr)) * 0.125, 0.0)
                W0[3, rows, :] = jnp.where(l0, ((ai - bi) - (ci - di)) * 0.125, 0.0)
                return _
            jax.lax.fori_loop(0, 256, body, 0, unroll=8)

        def qkv_prep(part):
            cp_q[part].wait()
            l32 = _iota((32, 128), 1)
            fld, rest = l32 >> 4, l32 & 15
            src = [32 * (rest >> 2) + 16 * ((rest >> 1) & 1) + 2 * ((fld - a) & 7) + (rest & 1) for a in range(8)]
            da = (l32 >> 1) & 7
            dr = (((l32 >> 4) & 3) << 2) | ((l32 >> 6) << 1) | (l32 & 1)
            dst = [(((da + j) & 7) << 4) | dr for j in range(8)]

            def body(q, _):
                def get(a):
                    return jnp.concatenate(
                        [pltpu.bitcast(wq_raw[pl.ds(pl.multiple_of(o + q * 32, 32), 32),
                                              pl.ds(D * part + 128 * a, 128)], u32) for o in (0, 512)], axis=0)
                v = [jnp.take_along_axis(get(a), src[a], axis=1) for a in range(8)]
                v = [v[(-j) % 8] for j in range(8)]
                for k in range(3):
                    m = ((fld >> k) & 1) == 1
                    v = [jnp.where(m, v[(j - (1 << k)) % 8], v[j]) for j in range(8)]
                v = [jnp.take_along_axis(v[j], dst[j], axis=1) for j in range(8)]
                rows = pl.ds(pl.multiple_of(q * 16, 16), 16)
                for j in range(4):
                    for n, w in enumerate(_strassen_rhs(v[j][:16], v[j + 4][:16], v[j][16:], v[j + 4][16:])):
                        Wq[n, rows, _cols(4 * part + j)] = w
                return _
            jax.lax.fori_loop(0, 16, body, 0)

        def wo_prep():
            cp_o.wait()
            for n in range(8):
                wo_u[n] = pltpu.bitcast(wo_raw[:, _cols(n)], u32)
            for n in range(4):
                for j in range(4):
                    for g1 in range(2):
                        for b in range(4):
                            quad = [wo_u[n + 4 * c, pl.ds(16 * b + 8 * g1 + j + 4 * r, 8, stride=64), :]
                                    for r in range(2) for c in range(2)]
                            for q, w in enumerate(_strassen_rhs(*quad)):
                                Wo[q, pl.ds(64 * j + 32 * g1 + 8 * b, 8), _cols(n)] = w

        def hook0():
            filter_prep(0)
            for cp in cp_q:
                cp.start()
            cp_o.start()
            filter_prep(1)

        def hook1():
            filter_prep(2)
            filter_prep(3)
            filter_pair()

        run_spectral([hook0, hook1, lambda: qkv_prep(0), lambda: (qkv_prep(1), qkv_prep(2), wo_prep())])

    pl.run_scoped(
        prologue,
        pltpu.VMEM((513, S), bf16), pltpu.VMEM((513, S), bf16),
        pltpu.VMEM((D, 3 * D), bf16), pltpu.VMEM((D, D), bf16), pltpu.VMEM((8, D // 2, 128), u32),
        pltpu.VMEM((2, 2, 256, 128), u32))

    def rowwise(last, ya, yb, ob, z0, z1, Q0, Q1, K0, K1, V0, V1):
        def idft_d(r0, c, gate):
            def get(ri):
                return jnp.concatenate(
                    [U[ri, c, pl.ds(r0 // 16 + g, 16, stride=PITCH), :] for g in range(T // 16)], axis=0)
            if c == 0:
                lo = _iota((T, 128), 1) < 64
                ur, ui = get(0), pltpu.roll(get(1), 64, 1)
                ya[:, 0:128] = _dot_nt(jnp.where(lo, ur, ui).astype(bf16), _b(gate(dm[0, 0:64, 0:128])))
                y = _dot_nt(jnp.where(lo, ui, ur).astype(bf16), _b(dm[0, 0:64, 128:256]))
                ya[:, 128:256] = y
            else:
                y = _dot_nt(jnp.concatenate([get(0), get(1)], axis=1).astype(bf16), _b(gate(dm[c])))
                ya[:, 256 * c:256 * (c + 1)] = y
            return y[0:8, 0:128]

        def ln_attn(r0, z, g, gate):
            zs = []
            for o in (0, H):
                rr = pl.ds(r0 + o + 16 * g, 16)
                yt = _tiles(ya[pl.ds(o + 16 * g, 16), :])
                yt[0] = gate(yt[0])
                x0 = X[rr, :] if last else xin[rr, :].astype(f32)
                xs = [a + b for a, b in zip(_tiles(x0), _radix8_inv(yt))]
                X[rr, :] = jnp.concatenate(xs, axis=1)
                zs.append(_layernorm(xs))
            for q, a in enumerate(_strassen_lhs(*zs)):
                w = _w(a)
                z[q, pl.ds(8 * g, 8), :] = w
            return w

        def strassen(A, B, n, put, gate):
            mm = lambda q: _dot(_b(A[q]), _b(gate(B[q, :, _cols(n)]) if q == 0 else B[q, :, _cols(n)]))
            m1, m2 = mm(0), mm(1)
            c22 = m1 - m2
            m3 = mm(2)
            put(1, 1, (c22 + m3) + mm(5))
            m4 = mm(3)
            c11 = m1 + m4
            put(1, 0, m2 + m4)
            m5 = mm(4)
            c11 = c11 - m5
            put(0, 1, m3 + m5)
            c11 = c11 + mm(6)
            put(0, 0, c11)
            return c11[0:8]

        def proj(z, qkv, n, gate):
            part, o = n // 4, 16 if n >= 4 else 0

            def put(r, c, y):
                qkv[part][4 * c + n % 4, pl.ds(o + r * H, H), :] = y
            return strassen(z, Wq, n, put, gate)

        def attend8(r0, qkv, rr, gate):
            Q, K, V = qkv
            q = [Q[j, pl.ds(rr, 8), :] for j in range(8)]
            q[0] = gate(q[0])
            L = []
            for w in range(8):
                p = _tree(jnp.add, [q[j] * K[j, pl.ds(16 + rr - 2 * w, 8), :] for j in range(8)])
                p = p + pltpu.roll(p, 64, 1)
                p = p + jnp.take_along_axis(p, lane ^ 1, axis=1)
                if rr < 2 * w:
                    p = jnp.where(r0 + rr + sub >= 2 * w, p, -1e9 * 32 ** 0.5)
                L.append(p)
            m = _tree(jnp.maximum, L)
            e = [jnp.exp2((l - m) * float(32 ** -0.5 * np.log2(np.e))) for l in L]
            inv = 1.0 / _tree(jnp.add, e)
            return [_tree(jnp.add, [e[w] * V[j, pl.ds(16 + rr - 2 * w, 8), :] for w in range(8)]) * inv
                    for j in range(8)]

        def attend(r0, qkv, g, gate):
            o = [[jnp.concatenate(p, axis=0) for p in zip(*[attend8(r0, qkv, h + 16 * g + e, gate) for e in (0, 8)])]
                 for h in (0, H)]
            for q, a in enumerate(_strassen_lhs(*o)):
                w = _w(a)
                ob[q, pl.ds(8 * g, 8), :] = w
            return w

        def out_proj(n, gate):
            def put(r, c, y):
                yb[pl.ds(r * H, H), _cols(4 * c + n)] = y
            return strassen(ob, Wo, n, put, gate)

        def residual(r0, g, gate):
            rr = pl.ds(r0 + 16 * g, 16)
            v = X[rr, :] + gate(yb[pl.ds(16 * g, 16), :])
            if last:
                xin[rr, :] = v.astype(bf16)
                return v
            X[rr, :] = v
            return ln_radix8(tb0, g, _tiles(v))

        def step(i, par, nxt, cur, prv):
            bufs = ((Q0, K0, V0), (Q1, K1, V1))
            new, old = bufs[par], bufs[1 - par]
            rn, rp = (i + 1) * T, (i - 1) * T
            if not isinstance(i, int):
                rn, rp = pl.multiple_of(rn, T), pl.multiple_of(rp, T)
            if cur:
                for j in range(8):
                    for dst, src in zip(new[1:], old[1:]):
                        dst[j, 0:16, :] = src[j, T:T + 16, :] if prv else jnp.zeros((16, 128), f32)
            m_n = [P_(idft_d, rn, c) for c in range(4)] if nxt else []
            m_c = [P_(proj, (z0, z1)[par], new, n) for n in range(12)] if cur else []
            m_o = [P_(out_proj, n) for n in range(4)] if prv else []
            m_d = [P_(dft_d, rp, tb0, c) for c in range(4)] if prv and not last else []
            mm = m_n + m_c[:9] + m_o + m_c[9:] + m_d
            a0 = len(m_n)
            a1 = a0 + len(m_c[:9])
            a2 = a1 + len(m_o)
            a3 = a2 + len(m_c[9:])
            vec = []
            if prv:
                vec += _spread([P_(attend, rp, old, g) for g in range(H // 16)], a0, a1)
            if nxt:
                vec += _spread([P_(ln_attn, rn, (z0, z1)[1 - par], g) for g in range(H // 16)],
                               a1 if prv else a0, a2 if prv else a1)
            if prv:
                vec += _spread([P_(residual, rp, g) for g in range(T // 16)], a2, a3)
            weave(mm, vec)
            if prv and last:
                out_copy(rp, i - 1).start()

        step(-1, 1, True, False, False)
        step(0, 0, True, True, False)

        def loop(i, _):
            for par in range(2):
                pl.when(i % 2 == par)(P_(step, i, par, True, True, True))
            return _
        jax.lax.fori_loop(1, NB - 1, loop, 0)
        step(NB - 1, 1, False, True, True)
        step(NB, 0, False, False, True)

    def run_rowwise(last):
        zs = pltpu.VMEM((7, H // 2, 512), u32)
        kv = pltpu.VMEM((8, 16 + T, 128), f32)
        pl.run_scoped(P_(rowwise, last), pltpu.VMEM((T, D), f32), pltpu.VMEM((T, D), f32), zs, zs, zs,
                      pltpu.VMEM((8, T, 128), f32), pltpu.VMEM((8, T, 128), f32), kv, kv, kv, kv)

    run_rowwise(False)
    run_spectral(None)
    run_rowwise(True)
    for i in range(NB):
        out_copy(i * T, i).wait()


@jax.jit
def pallas_interleave_layers__spectral_gfnet__sliding_local_dilated__prompt_kernel(A_x, A_w_r, A_w_i, B_x, B_wqkv, B_wo):
    del B_x
    hbm = pl.BlockSpec(memory_space=pltpu.HBM)
    args = (A_x.reshape(S, D), A_w_r.T, A_w_i.T, B_wqkv, B_wo, jnp.asarray(_seeds()))
    out = pl.pallas_call(
        _kernel,
        out_shape=jax.ShapeDtypeStruct((S, D), bf16),
        in_specs=[hbm] * 6,
        out_specs=hbm,
        scratch_shapes=[
            pltpu.VMEM((34, 8, 128), f32),
            pltpu.VMEM((S, D), bf16),
            pltpu.VMEM((S, D), f32),
            pltpu.VMEM((4, 16 * PITCH, 128), u32),
            pltpu.VMEM((2, 4, 16 * PITCH, 128), f32),
            pltpu.VMEM((4, 128, 256), u32),
            pltpu.VMEM((16, 128, 256), u32),
            pltpu.VMEM((16, 128, 256), u32),
            pltpu.VMEM((3, S, 128), u32),
            pltpu.VMEM((4, S, 128), f32),
            pltpu.VMEM((7, 256, 1536), u32),
            pltpu.VMEM((7, 256, 512), u32),
            pltpu.VMEM((T // 2, D), u32),
            pltpu.VMEM((T // 2, D), u32),
            pltpu.SemaphoreType.DMA((NB + 13,)),
        ],
        compiler_params=pltpu.CompilerParams(vmem_limit_bytes=120 * 1024 * 1024),
    )(*[pltpu.with_memory_space_constraint(a, pltpu.HBM) for a in args])
    return out.reshape(1, S, D)
```

```python
import functools
import numpy as np
import jax
import jax.numpy as jnp
from jax.experimental import pallas as pl
from jax.experimental.pallas import tpu as pltpu

S, D = 2048, 1024
f32, bf16, u32 = jnp.float32, jnp.bfloat16, jnp.uint32
T = 256
NB = S // T
H = T // 2
PITCH = 129
WROWS = 264
R2 = float(np.sqrt(0.5))
C8, S8 = float(np.cos(np.pi / 8)), float(np.sin(np.pi / 8))
SCALE = 2.0 / (S * D)


def _seeds():
    r = np.arange(8)[:, None]
    l = np.arange(128)[None, :]
    cls, j = l >> 6, l & 63
    tiles = []
    freqs = [8 * j, 8 * j + 4] + [8 * j + np.where(cls == 0, c, 8 - c) for c in (1, 2, 3)]
    for m in freqs:
        th, st = 2 * np.pi * r * m / D, 2 * np.pi * 8 * m / D + 0 * r
        tiles += [np.cos(th), np.sin(th), np.cos(st), np.sin(st)]
    for h in range(2):
        col = 128 * h + l
        b, odd = col >> 1, (col & 1) == 1
        al, st, tw = 2 * np.pi * r * b / 128, 2 * np.pi * 8 * b / 128 + 0 * r, 2 * np.pi * b / S + 0 * r
        tiles += [np.where(odd, np.sin(al), np.cos(al)), np.where(odd, np.cos(al), -np.sin(al)),
                  np.cos(st), np.sin(st), np.cos(tw), np.sin(tw)]
    tw = 2 * np.pi * r / S + 0 * l
    tiles += [np.cos(tw), np.sin(tw)]
    return np.stack(tiles).astype(np.float32)


def _iota(shape, axis):
    return jax.lax.broadcasted_iota(jnp.int32, shape, axis)


def _pack(a, b):
    return pltpu.pack_elementwise([a, b], packed_dtype=bf16)


def _unpack(w, i):
    return pltpu.unpack_elementwise(w, index=i, packed_dtype=bf16, unpacked_dtype=f32)


def _tiles(v):
    return [v[:, 128 * a:128 * (a + 1)] for a in range(v.shape[1] // 128)]


def _tree(op, xs):
    xs = list(xs)
    while len(xs) > 1:
        xs = [op(xs[i], xs[i + 1]) if i + 1 < len(xs) else xs[i] for i in range(0, len(xs), 2)]
    return xs[0]


def _rot(c, s, cs, ss):
    return c * cs - s * ss, s * cs + c * ss


def _layernorm(xs):
    m = jnp.sum(_tree(jnp.add, xs), axis=-1, keepdims=True) * (1.0 / D)
    xc = [x - m for x in xs]
    v = jnp.sum(_tree(jnp.add, [x * x for x in xc]), axis=-1, keepdims=True) * (1.0 / D)
    inv = jax.lax.rsqrt(v + 1e-5)
    return [x * inv for x in xc]


def _radix8_fwd(z):
    e = [z[a] + z[a + 4] for a in range(4)]
    o = [z[a] - z[a + 4] for a in range(4)]
    s02, s13 = e[0] + e[2], e[1] + e[3]
    p, q = (o[1] - o[3]) * R2, (o[1] + o[3]) * R2
    return [s02 + s13, s02 - s13, o[0] + p, o[2] + q, e[0] - e[2], e[3] - e[1], o[0] - p, o[2] - q]


def _radix8_inv(t):
    t0, t4, r1, n1, r2, i2, r3, i3 = t
    a, b = t0 + t4, t0 - t4
    E = [a + r2, b - i2, a - r2, b + i2]
    u, v = r1 - r3, i3 - n1
    O = [r1 + r3, (u - v) * R2, i3 + n1, (u + v) * (-R2)]
    return [E[k] + O[k] for k in range(4)] + [E[k] - O[k] for k in range(4)]


def _dft4(x, sgn):
    (ar, ai), (br, bi), (cr, ci), (dr, di) = x
    sr, si, tr, ti = ar + cr, ai + ci, ar - cr, ai - ci
    ur, ui, vr, vi = br + dr, bi + di, br - dr, bi - di
    y1, y3 = (tr + vi, ti - vr), (tr - vi, ti + vr)
    if sgn > 0:
        y1, y3 = y3, y1
    return [(sr + ur, si + ui), y1, (sr - ur, si - ui), y3]


def _tw16(x, k, sgn):
    xr, xi = x
    k = k % 16
    if k == 0:
        return x
    if k == 4:
        return (xi, -xr) if sgn < 0 else (-xi, xr)
    if k == 2:
        return ((xr + xi) * R2, (xi - xr) * R2) if sgn < 0 else ((xr - xi) * R2, (xi + xr) * R2)
    if k == 6:
        return ((xi - xr) * R2, (xr + xi) * (-R2)) if sgn < 0 else ((xr + xi) * (-R2), (xr - xi) * R2)
    c, s = float(np.cos(np.pi * k / 8)), float(sgn * np.sin(np.pi * k / 8))
    return (xr * c - xi * s, xi * c + xr * s)


def _dft16(x, sgn):
    cols = [_dft4([x[a2 + 4 * a1] for a1 in range(4)], sgn) for a2 in range(4)]
    out = [None] * 16
    for k1 in range(4):
        y = _dft4([_tw16(cols[a2][k1], a2 * k1, sgn) for a2 in range(4)], sgn)
        for k2 in range(4):
            out[k1 + 4 * k2] = y[k2]
    return out


def _dot(a, b):
    return jnp.dot(a, b, preferred_element_type=f32)


def _dot_nt(a, b):
    return jax.lax.dot_general(a, b, (((1,), (1,)), ((), ())), preferred_element_type=f32)


def _b(w):
    return pltpu.bitcast(w, bf16)


def _w(v):
    return pltpu.bitcast(v.astype(bf16), u32)


def _strassen_lhs(top, bot):
    a11, a12 = jnp.concatenate(top[:4], axis=1), jnp.concatenate(top[4:], axis=1)
    a21, a22 = jnp.concatenate(bot[:4], axis=1), jnp.concatenate(bot[4:], axis=1)
    return [a11 + a22, a21 + a22, a11, a22, a11 + a12, a21 - a11, a12 - a22]


def _strassen_rhs(b11, b12, b21, b22):
    def comb(p, q, op):
        return _pack(op(_unpack(p, 0), _unpack(q, 0)), op(_unpack(p, 1), _unpack(q, 1)))
    return [comb(b11, b22, jnp.add), b11, comb(b12, b22, jnp.subtract), comb(b21, b11, jnp.subtract),
            b22, comb(b11, b12, jnp.add), comb(b21, b22, jnp.add)]


def _weave(never, mm, vec):
    def gate(tokens):
        def apply(v):
            if not tokens:
                return v
            t = v[0:8, 0:128]
            tok = _tree(jnp.bitwise_or, [k if k.dtype == u32 else pltpu.bitcast(k, u32) for k in tokens])
            t = jnp.where(never, tok if t.dtype == u32 else pltpu.bitcast(tok, t.dtype), t)
            if v.shape[1] > 128:
                t = jnp.concatenate([t, v[0:8, 128:]], axis=1)
            return jnp.concatenate([t, v[8:]], axis=0) if v.shape[0] > 8 else t
        return apply
    done, due = {}, {}
    for n in range(-1, len(mm)):
        if n >= 0:
            done[n] = mm[n](gate(due.pop(n, [])))
        for job, after, before in vec:
            if max(after, -1) == n:
                tied = before is not None
                tok = job(gate([done[n]] if tied and n >= 0 else []))
                if tied:
                    due.setdefault(before, []).append(tok[0:8, 0:128])


def _spread(jobs, lo, hi, window=None):
    out = []
    for k, job in enumerate(jobs):
        n = lo + (k * (hi - lo)) // len(jobs)
        out.append((job, n - 1, None if window is None else min(n + window, hi)))
    return out


def _cols(j, n=1):
    return pl.ds(128 * j, 128 * n)


def _kernel(x_hbm, wr_hbm, wi_hbm, wqkv_hbm, wo_hbm, seed_hbm, out_hbm,
            seed, xin, X, X2, Vp, U, dm, G, Gi, Wf, Wq, Wo, tb0, tb1, wr, wi, wq_raw, wo_raw, tmp, WE, sem):
    P_ = functools.partial
    sub = _iota((8, 128), 0)
    lane = _iota((8, 128), 1)
    lane16 = _iota((16, 128), 1)

    def x_copy(i):
        return pltpu.make_async_copy(x_hbm.at[pl.ds(i * T, T)], xin.at[pl.ds(i * T, T)], sem.at[i])

    def out_copy(r0, i):
        return pltpu.make_async_copy(xin.at[pl.ds(r0, T)], out_hbm.at[pl.ds(r0, T)], sem.at[i])

    cp_seed = pltpu.make_async_copy(seed_hbm, seed, sem.at[NB])
    cp_w = [pltpu.make_async_copy(src.at[:, pl.ds(1024 * n, 1024)], dst.at[:, pl.ds(1024 * n, 1024)],
                                  sem.at[NB + 1 + 2 * n + q])
            for n in range(2) for q, (src, dst) in enumerate(((wr_hbm, wr), (wi_hbm, wi)))]
    cp_q = [pltpu.make_async_copy(wqkv_hbm.at[:, pl.ds(D * n, D)], wq_raw.at[:, pl.ds(D * n, D)],
                                  sem.at[NB + 5 + n]) for n in range(3)]
    cp_o = pltpu.make_async_copy(wo_hbm, wo_raw, sem.at[NB + 8])
    cp_seed.start()
    for i in range(NB):
        x_copy(i).start()
    cp_seed.wait()

    zero = (seed[0] > 2.0).astype(jnp.int32)[0, 0]
    zero8 = pl.multiple_of(8 * zero, 8)
    regions = []

    def region(fn):
        regions.append(fn)
        pl.when(zero < len(regions))(fn)

    def weave(mm, vec):
        _weave(seed[0] > 2.0, mm, vec)

    def gen_dm():
        lo = lane16 < 64
        for n in range(5):
            c, s, cs, ss = (seed[4 * n + q] for q in range(4))
            for g in range(8):
                c2, s2 = _rot(c, s, cs, ss)
                cc, sc = jnp.concatenate([c, c2], axis=0), jnp.concatenate([s, s2], axis=0)
                rows, rows2 = pl.ds(8 * g, 8), pl.ds(64 + 8 * g, 8)
                if n == 0:
                    alt = (1 - 2 * (_iota((16, 128), 0) & 1)).astype(f32)
                    dm[0, rows, 0:128] = _w(jnp.where(lane16 == 64, alt, jnp.where(lo, cc, -sc)))
                elif n == 1:
                    dm[0, rows, 128:256] = _w(jnp.where(lo, -sc, cc))
                else:
                    sg = jnp.where(lo, 1.0, -1.0) * (-1.0 if n == 2 else 1.0)
                    dm[n - 1, rows, 0:128] = _w(cc)
                    dm[n - 1, rows, 128:256] = _w(-sc)
                    dm[n - 1, rows2, 0:128] = _w(sg * sc)
                    dm[n - 1, rows2, 128:256] = _w(sg * cc)
                if g < 7:
                    c, s = _rot(c2, s2, cs, ss)

    def gen_g(inverse):
        st = dict(pq=[seed[20], seed[21], seed[26], seed[27]], tw=(seed[32], seed[33]))
        c1, s1 = float(np.cos(2 * np.pi * 8 / S)), float(np.sin(2 * np.pi * 8 / S))

        def job(g, gate):
            rows, rows2 = pl.ds(8 * g, 8), pl.ds(64 + 8 * g, 8)
            tw1 = _rot(*st['tw'], c1, s1)
            cb, sb = (jnp.concatenate(v, axis=0) for v in zip(st['tw'], tw1))
            st['tw'] = _rot(*tw1, c1, s1)
            for h in range(2):
                p0, q0 = st['pq'][2 * h:2 * h + 2]
                cs, ss, ct, sn = (seed[22 + 6 * h + n] for n in range(4))
                q1, p1 = _rot(q0, p0, cs, ss)
                p, q = jnp.concatenate([p0, p1], axis=0), jnp.concatenate([q0, q1], axis=0)
                st['pq'][2 * h + 1], st['pq'][2 * h] = _rot(q1, p1, cs, ss)
                if inverse:
                    sg = (1 - 2 * (lane16 & 1)).astype(f32) * SCALE
                    p, q = p * sg, q * (-sg)
                    ct, sn = jnp.concatenate([ct, ct], axis=0), jnp.concatenate([sn, sn], axis=0)
                dst = Gi if inverse else G
                for a in range(16):
                    dst[a, rows, _cols(h)] = _w(p)
                    dst[a, rows2, _cols(h)] = _w(q)
                    if a < 15 and inverse:
                        p, q = _rot(p, q, ct, sn)
                    elif a < 15:
                        q, p = _rot(q, p, cb, sb)
        return [P_(job, g) for g in range(8)]

    def filter_tile(t, c, gate):
        we = WE.at[t]
        if c == 1:
            a = pltpu.bitcast(wr[0:512, _cols(t)], u32)
            b = pltpu.bitcast(wi[0:512, _cols(t)], u32)
            we[0:256] = (a & 0xFFFF) | (b << 16)
            we[256:512] = (a >> 16) | (b & jnp.uint32(0xFFFF0000))
        w = jnp.concatenate([we[pl.ds(256 * (r & 1) + (r >> 1), 64, stride=4), :]
                             for r in (c, (8 - c) if c else 4)], axis=0)
        if c == 0:
            def rows(src_t):
                return [jnp.broadcast_to(src[m:m + 1, _cols(src_t)].astype(f32), (8, 128))
                        for m in (0, D // 2) for src in (wr, wi)]
            ar, ai, br, bi = rows(t)
            cr, ci, dr, di = (jnp.take_along_axis(jnp.where(lane == 0, p, q), (128 - lane) & 127, axis=1)
                              for p, q in zip(rows((16 - t) % 16), rows(15 - t)))
            same = _pack(((ar + br) + (cr + dr)) * 0.125, ((ai + bi) - (ci + di)) * 0.125)
            pair = _pack(((ar - br) + (cr - dr)) * 0.125, ((ai - bi) - (ci - di)) * 0.125)
            w = jnp.concatenate([jnp.where(sub == 0, same, w[0:8]), w[8:]], axis=0)
            p = jnp.concatenate([jnp.where(sub == 0, pair, 0), jnp.zeros((120, 128), u32)], axis=0)
            Wf[4, pl.ds(128 * t, 128), :] = p.T
        Wf[c, pl.ds(128 * t, 128), :] = w.T

    def qkv_jobs(part):
        x8 = lambda v: jnp.concatenate([v] * 8, axis=0)

        def spin(a, gate):
            l = lane
            src = x8(32 * ((l >> 2) & 3) + 16 * ((l >> 1) & 1) + 2 * (((l >> 4) - a) & 7) + (l & 1))
            for r in range(8):
                w = pltpu.bitcast(wq_raw[pl.ds(128 * r, 128), pl.ds(D * part + 128 * a, 128)], u32)
                tmp[a, pl.ds(64 * r, 64), :] = jnp.take_along_axis(w, src, axis=1)

        def gather(j, gate):
            l = lane
            rest = (((l >> 4) & 3) << 2) | ((l >> 6) << 1) | (l & 1)

            def col(jj, r0):
                v = tmp[0, pl.ds(r0, 64), :]
                for a in range(1, 8):
                    v = jnp.where(x8(l >> 4) == ((jj + a) & 7), tmp[a, pl.ds(r0, 64), :], v)
                return jnp.take_along_axis(v, x8(((((l >> 1) + jj) & 7) << 4) | rest), axis=1)
            for r in range(4):
                b11, b21 = col(j, 64 * r), col(j, 256 + 64 * r)
                b12, b22 = col(j + 4, 64 * r), col(j + 4, 256 + 64 * r)
                for n, w in enumerate(_strassen_rhs(b11, b12, b21, b22)):
                    Wq[n, pl.ds(64 * r, 64), _cols(4 * part + j)] = w
        return [P_(spin, a) for a in range(8)] + [P_(gather, j) for j in range(4)]

    def wo_jobs():
        def stage(n, gate):
            w = pltpu.bitcast(wo_raw[:, _cols(n)], u32)
            for a in range(8):
                tmp[n, pl.ds(65 * a, 64), :] = w[64 * a:64 * a + 64]

        def gather(n, gate):
            for j in range(4):
                for g1 in range(2):
                    for b in range(4):
                        quad = [tmp[n + 4 * c, pl.ds(16 * b + 8 * g1 + j + 4 * r, 8, stride=65), :]
                                for r in range(2) for c in range(2)]
                        for q, w in enumerate(_strassen_rhs(*quad)):
                            Wo[q, pl.ds(64 * j + 32 * g1 + 8 * b, 8), _cols(n)] = w
        return [P_(stage, n) for n in range(8)] + [P_(gather, n) for n in range(4)]

    def ln_radix8(tb, g, xs):
        w = _w(jnp.concatenate(_radix8_fwd(_layernorm(xs)), axis=1))
        tb[pl.ds(8 * g, 8), :] = w
        return w

    def dft_d(r0, tb, c, gate):
        if c == 0:
            a = _dot(_b(tb[:, 0:128]), _b(gate(dm[0, 0:64, 0:128])))
            b = _dot(_b(tb[:, 128:256]), _b(dm[0, 0:64, 128:256]))
            lo = _iota((T, 128), 1) < 64
            w = _pack(jnp.where(lo, a, b), pltpu.roll(jnp.where(lo, b, a), 64, 1))
        else:
            y = _dot(_b(tb[:, 256 * c:256 * (c + 1)]), _b(gate(dm[c])))
            w = _pack(y[:, :128], y[:, 128:])
        for g in range(T // 8):
            Vp[c, pl.ds((g % 2) * 8 * PITCH + r0 // 16 + g // 2, 8, stride=PITCH), :] = w[8 * g:8 * g + 8, :]
        return w[0:8]

    def spectral(first, *R):
        def mm1(c, a, gate):
            v = Vp[c, pl.ds(a * PITCH, 128), :]
            if c == 0:
                R[c][a, 0:256, :] = _dot(_b(G[a]), _b(v))
            else:
                for h in range(2):
                    R[c][a, pl.ds(256 * h, 256), :] = _dot(_b(G[a, :, _cols(h)]), _b(v[64 * h:64 * h + 64]))

        def mid(c, g, gate):
            def load(a, r):
                v = R[c][a, pl.ds(r, 8), :]
                return v + R[c][a, pl.ds(256 + r, 8), :] if c else v
            y = _dft16([(load(a, 8 * g), load(a, 128 + 8 * g)) for a in range(16)], -1)
            if c == 0:
                part = []
                for a in range(16):
                    w1 = [load(a, o + 8 * (15 - g)) for o in (0, 128)]
                    w0 = [load(a, o + 8 * ((16 - g) % 16)) for o in (0, 128)]
                    if g == 0:
                        w0 = _tw16(w0, a, -1)
                    part.append(tuple(jnp.take_along_axis(jnp.where(sub == 0, p, q), (8 - sub) & 7, axis=0)
                                      for p, q in zip(w0, w1)))
                yneg = _dft16(part, -1)
            z = []
            for k1 in range(16):
                yr, yi = y[k1]
                w = Wf[c, pl.ds(128 * k1 + 8 * g, 8), :]
                ar, ai = _unpack(w, 0), _unpack(w, 1)
                zr, zi = yr * ar - yi * ai, yr * ai + yi * ar
                if c == 0:
                    w = Wf[4, pl.ds(128 * k1 + 8 * g, 8), :]
                    br, bi = _unpack(w, 0), _unpack(w, 1)
                    pr, pi = yneg[15 - k1]
                    zr, zi = zr + (pr * br + pi * bi), zi + (pr * bi - pi * br)
                z.append((zr, zi))
            for a, v in enumerate(_dft16(z, 1)):
                w = pltpu.bitcast(_pack(*v), f32)
                R[c][a, pl.ds(zero8 + 512 + 8 * g, 8), :] = w
            if g == 15 and c < 3 and not first:
                R[c + 1][0, pl.ds(zero8 + 640, 8), :] = w

        def mm2(c, a, gate):
            v = pltpu.bitcast(R[c][a, 512:640, :], u32)
            for h in range(2):
                u = _dot(_b(Gi[a, :, _cols(h)]), _b(v[64 * h:64 * h + 64]))
                U[2 * h, c, pl.ds(a * PITCH, 128), :] = u[:128]
                U[2 * h + 1, c, pl.ds(a * PITCH, 128), :] = u[128:]

        m1 = lambda c: [P_(mm1, c, a) for a in range(16)]
        m2 = lambda c: [P_(mm2, c, a) for a in range(16)]
        mids = lambda c: [P_(mid, c, g) for g in range(16)]

        def run(mm, vec, before=None):
            def fn():
                if before:
                    before()
                weave(mm, _spread(vec() if callable(vec) else vec, 0, len(mm)))
            region(fn)

        if first:
            def wait_w(n):
                cp_w[2 * n].wait()
                cp_w[2 * n + 1].wait()

            def start_q():
                for cp in cp_q + [cp_o]:
                    cp.start()
            run(m1(0), lambda: gen_g(True))
            run(m1(1), [P_(filter_tile, t, c) for t in range(8) for c in (1, 2, 3)],
                lambda: (wait_w(0), start_q()))
            run(m1(2), [P_(filter_tile, t, c) for u in range(8, 16) for t, c in ((u, 1), (u, 2), (u, 3), (u - 8, 0), (u, 0))], lambda: wait_w(1))
            run(m1(3), mids(1))
            run(m2(1), mids(2))
            run(m2(2), mids(3))
            q = qkv_jobs(0)
            run(m2(3), [j for g, m in enumerate(mids(0)) for j in [m] + ([q[g // 2]] if g % 2 else [])],
                cp_q[0].wait)
            run(m2(0), q[8:])
        else:
            run(m1(0), [])
            v = mids(0) + mids(1) + mids(2) + mids(3)
            c0, c1, c2 = map(int, '16,42,53'.split(','))
            run(m1(1) + m1(2), v[:c0])
            run(m1(3) + m2(0), v[c0:c1])
            run(m2(1), v[c1:c2])
            run(m2(2), v[c2:])
            run(m2(3), [])

    def run_spectral(first):
        pl.run_scoped(P_(spectral, first), *[pltpu.VMEM((16, 648, 128), f32)] * 4)

    def rowwise(last, ya, yb, zf, o0, o1, z0, z1, QK0, QK1, VO0, VO1):
        bufs = ((QK0, VO0), (QK1, VO1))

        def idft_d(r0, ya, c, gate):
            def get(q):
                return jnp.concatenate(
                    [U[q, c, pl.ds(r0 // 16 + g, 16, stride=PITCH), :]
                     + U[q + 2, c, pl.ds(r0 // 16 + g, 16, stride=PITCH), :] for g in range(T // 16)], axis=0)
            if c == 0:
                lo = _iota((T, 128), 1) < 64
                ur, ui = get(0), pltpu.roll(get(1), 64, 1)
                ya[:, 0:128] = _dot_nt(jnp.where(lo, ur, ui).astype(bf16), _b(gate(dm[0, 0:64, 0:128])))
                y = _dot_nt(jnp.where(lo, ui, ur).astype(bf16), _b(dm[0, 0:64, 128:256]))
                ya[:, 128:256] = y
            else:
                y = _dot_nt(jnp.concatenate([get(0), get(1)], axis=1).astype(bf16), _b(gate(dm[c])))
                ya[:, 256 * c:256 * (c + 1)] = y
            return y[0:8, 0:128]

        def ln_attn(r0, ya, g, gate):
            rr, rows = pl.ds(r0 + 16 * g, 16), pl.ds(16 * g, 16)
            yt = _tiles(ya[rows, :])
            yt[0] = gate(yt[0])
            x0 = X2[rr, :] if last else xin[rr, :].astype(f32)
            xs = [a + b for a, b in zip(_tiles(x0), _radix8_inv(yt))]
            X[rr, :] = jnp.concatenate(xs, axis=1)
            z = jnp.concatenate(_layernorm(xs), axis=1)
            zf[rows, :] = z
            return z

        def operands(get, dst, g, gate):
            top, bot = get(pl.ds(16 * g, 16)), get(pl.ds(H + 16 * g, 16))
            top[0] = gate(top[0])
            for q, a in enumerate(_strassen_lhs(top, bot)):
                w = _w(a)
                dst[q, pl.ds(8 * g, 8), :] = w
            return w

        def strassen(A, B, n, put, gate):
            mm = lambda q: _dot(_b(A[q]), _b(gate(B[q, :, _cols(n)]) if q == 0 else B[q, :, _cols(n)]))
            m1, m2 = mm(0), mm(1)
            c22 = m1 - m2
            m3 = mm(2)
            put(1, 1, (c22 + m3) + mm(5))
            m4 = mm(3)
            c11 = m1 + m4
            put(1, 0, m2 + m4)
            m5 = mm(4)
            c11 = c11 - m5
            put(0, 1, m3 + m5)
            c11 = c11 + mm(6)
            put(0, 0, c11)
            return c11[0:8]

        def proj(z, par, n, gate):
            part = n // 4
            dst, t0 = bufs[par][part >> 1], 8 * (part & 1)

            def put(r, c, y):
                dst[t0 + 4 * c + n % 4, pl.ds(16 + r * H, H), :] = y
            return strassen(z, Wq, n, put, gate)

        def softmax(r0, par, rr, gate):
            QK = bufs[par][0]
            q = [QK[j, pl.ds(16 + rr, 8), :] for j in range(8)]
            q[0] = gate(q[0])
            L = []
            for w in range(8):
                p = _tree(jnp.add, [q[j] * QK[8 + j, pl.ds(16 + rr - 2 * w, 8), :] for j in range(8)])
                p = p + pltpu.roll(p, 64, 1)
                p = p + jnp.take_along_axis(p, lane ^ 1, axis=1)
                if rr < 2 * w:
                    p = jnp.where(r0 + rr + sub >= 2 * w, p, -1e9 * 32 ** 0.5)
                L.append(p)
            m = _tree(jnp.maximum, L)
            e = [jnp.exp2((l - m) * float(32 ** -0.5 * np.log2(np.e))) for l in L]
            inv = 1.0 / _tree(jnp.add, e)
            return [v * inv for v in e]

        def mix(par, rr, z8, p):
            VO = bufs[par][1]
            for j in range(8):
                o = _tree(jnp.add, [p[w] * VO[j, pl.ds(16 + rr - 2 * w, 8), :] for w in range(8)])
                VO[8 + j, pl.ds(z8 + rr, 8), :] = o
            return o

        def attend(r0, par, rr, ordered, gate):
            p = softmax(r0, par, rr, gate)
            if ordered:
                QK = bufs[par][0]
                for w in range(8):
                    QK[16 + w, pl.ds(zero8 + rr, 8), :] = p[w]
                p = [QK[16 + w, pl.ds(rr, 8), :] for w in range(8)]
            return mix(par, rr, zero8 if ordered else 0, p)

        def out_proj(r0, ob, yb, n, gate):
            def put(r, c, y):
                at = (pl.ds(r0 + r * H, H), _cols(4 * c + n))
                if last:
                    xin[at] = (X[at] + y).astype(bf16)
                else:
                    yb[pl.ds(r * H, H), _cols(4 * c + n)] = X[at] + y
            return strassen(ob, Wo, n, put, gate)

        def residual(r0, tb, yb, g, gate):
            v = gate(yb[pl.ds(16 * g, 16), :])
            X2[pl.ds(r0 + 16 * g, 16), :] = v
            return ln_radix8(tb, g, _tiles(v))

        def fourfold(fn, gate):
            return [fn(c, gate if c == 0 else (lambda v: v)) for c in range(4)][-1]
        m_idft = lambda r0, y=ya: [P_(fourfold, P_(idft_d, r0, y))]
        m_proj = lambda par: [P_(proj, (z0, z1)[par], par, n) for n in range(12)]
        m_out = lambda r0, par, y=yb: [P_(out_proj, r0, (o0, o1)[par], y, n) for n in range(4)]
        m_dft = lambda r0, tb=tb0: [] if last else [P_(fourfold, P_(dft_d, r0, tb))]

        def v_ln(r0, par, y=ya):
            jobs = []
            for g in range(H // 16):
                jobs += [P_(ln_attn, r0, y, g), P_(ln_attn, r0, y, g + H // 16),
                         P_(operands, lambda rows: _tiles(zf[rows, :]), (z0, z1)[par], g)]
            return jobs

        def v_att(r0, par, ordered=True):
            jobs = []
            for g in range(H // 16):
                jobs += [P_(attend, r0, par, h + 16 * g + e, ordered) for h in (0, H) for e in (0, 8)]
                jobs += [P_(operands, lambda rows: [bufs[par][1][8 + j, rows, :] for j in range(8)],
                            (o0, o1)[par], g)]
            return jobs
        v_res = lambda r0, tb=tb0, y=yb: [] if last else [P_(residual, r0, tb, y, g) for g in range(T // 16)]

        def halo(par, first=False):
            for j in range(8):
                for dst, src, t in zip(bufs[par], bufs[1 - par], (8 + j, j)):
                    dst[t, 0:16, :] = jnp.zeros((16, 128), f32) if first else src[t, T:T + 16, :]

        def head0():
            halo(0, True)
            weave(m_idft(0, yb) + m_idft(T), _spread(v_ln(0, 0, yb), 1, 2))

        def head(part):
            vec = []
            if not last:
                (cp_q[1], cp_q[2], cp_o)[part].wait()
                vec = _spread(qkv_jobs(part + 1) if part < 2 else wo_jobs(), 0, 4)
            if part == 2 or last:
                jobs = v_ln(T, 1)
                vec = vec + _spread(jobs[8 * part:8 * part + 8] if last else jobs, 0, 4)
            weave(m_proj(0)[4 * part:4 * part + 4], vec)

        def step(i, par, nxt=True, old=True):
            rn, rp, ro = ((i + d) * T if isinstance(i, int) else pl.multiple_of((i + d) * T, T) for d in (1, -1, -2))
            halo(par)
            mo, mi = m_out(ro, par) if old else [], m_idft(rn) if nxt else []
            a, b = len(mo), len(mo) + len(mi)
            na, nl, wl = (11, 11, 2) if last else (12, 12, 1)
            vec = _spread(v_att(rp, 1 - par), 0, b + na - (0 if old or last else 1), 2)
            if old:
                vec += _spread(v_res(ro), a + 0, b + 12, 1)
            if nxt:
                vec += _spread(v_ln(rn, 1 - par), b + 0, b + nl - (0 if old or last else 1), wl)
            weave(mo + mi + m_proj(par) + (m_dft(ro) if old else []), vec)
            if last and old:
                out_copy(ro, i - 2).start()

        def tail1():
            r6, r7 = (NB - 2) * T, (NB - 1) * T
            weave(m_out(r6, 0), _spread(v_att(r7, 1, False), 0, 4, 1))
            if last:
                out_copy(r6, NB - 2).start()

        def tail2():
            r6, r7 = (NB - 2) * T, (NB - 1) * T
            for job in v_res(r6):
                job(lambda v: v)
            weave(m_out(r7, 1, ya) + m_dft(r6), [])
            if last:
                out_copy(r7, NB - 1).start()
            for job in v_res(r7, tb1, ya):
                job(lambda v: v)
            weave(m_dft(r7, tb1), [])

        for fn in (head0, P_(head, 0), P_(head, 1), P_(head, 2), P_(step, 1, 1, True, False)):
            region(fn)

        def loop(i, _):
            for par in range(2):
                pl.when(i % 2 == par)(P_(step, i, par))
            return _
        jax.lax.fori_loop(2, NB - 1, loop, 0)
        for fn in (P_(step, NB - 1, 1, False), tail1, tail2):
            region(fn)

    def run_rowwise(last):
        zs = pltpu.VMEM((7, H // 2, 512), u32)
        rows, qk, vo = pltpu.VMEM((T, D), f32), pltpu.VMEM((24, 16 + T, 128), f32), pltpu.VMEM((16, 16 + T, 128), f32)
        pl.run_scoped(P_(rowwise, last), rows, rows, rows, zs, zs, zs, zs, qk, qk, vo, vo)

    gen_dm()

    def ln_x(i, g, gate):
        return ln_radix8((tb0, tb1)[i % 2], g, _tiles(xin[pl.ds(i * T + 16 * g, 16), :].astype(f32)))

    def first_dft(i):
        vec = []
        if i + 1 < NB:
            x_copy(i + 1).wait()
            if i + 1 == NB - 2:
                for cp in cp_w:
                    cp.start()
            vec = [P_(ln_x, i + 1, g) for g in range(T // 16)]
        mm = [P_(dft_d, i * T, (tb0, tb1)[i % 2], c) for c in range(4)] if i >= 0 else []
        if i + 1 < NB:
            weave(mm, _spread(vec, 0, len(mm), 2))
        else:
            weave(mm, _spread(gen_g(False), 0, len(mm)))

    for i in range(-1, NB):
        region(P_(first_dft, i))
    run_spectral(True)
    run_rowwise(False)
    run_spectral(False)
    run_rowwise(True)
    for i in range(NB):
        out_copy(i * T, i).wait()


@jax.jit
def pallas_interleave_layers__spectral_gfnet__sliding_local_dilated__prompt_kernel(A_x, A_w_r, A_w_i, B_x, B_wqkv, B_wo):
    del B_x
    hbm = pl.BlockSpec(memory_space=pltpu.HBM)
    args = (A_x.reshape(S, D), A_w_r.T, A_w_i.T, B_wqkv, B_wo, jnp.asarray(_seeds()))
    out = pl.pallas_call(
        _kernel,
        out_shape=jax.ShapeDtypeStruct((S, D), bf16),
        in_specs=[hbm] * 6,
        out_specs=hbm,
        scratch_shapes=[
            pltpu.VMEM((34, 8, 128), f32),
            pltpu.VMEM((S, D), bf16),
            pltpu.VMEM((S, D), f32),
            pltpu.VMEM((S, D), f32),
            pltpu.VMEM((4, 16 * PITCH, 128), u32),
            pltpu.VMEM((4, 4, 16 * PITCH, 128), f32),
            pltpu.VMEM((4, 128, 256), u32),
            pltpu.VMEM((16, 128, 256), u32),
            pltpu.VMEM((16, 128, 256), u32),
            pltpu.VMEM((5, S, 128), u32),
            pltpu.VMEM((7, 256, 1536), u32),
            pltpu.VMEM((7, 256, 512), u32),
            pltpu.VMEM((T // 2, D), u32),
            pltpu.VMEM((T // 2, D), u32),
            pltpu.VMEM((513, S), bf16),
            pltpu.VMEM((513, S), bf16),
            pltpu.VMEM((D, 3 * D), bf16),
            pltpu.VMEM((D, D), bf16),
            pltpu.VMEM((8, 520, 128), u32),
            pltpu.VMEM((16, 512, 128), u32),
            pltpu.SemaphoreType.DMA((NB + 9,)),
        ],
        compiler_params=pltpu.CompilerParams(vmem_limit_bytes=120 * 1024 * 1024),
    )(*[pltpu.with_memory_space_constraint(a, pltpu.HBM) for a in args])
    return out.reshape(1, S, D)
```

```python
import functools
import numpy as np
import jax
import jax.numpy as jnp
from jax.experimental import pallas as pl
from jax.experimental.pallas import tpu as pltpu

S, D = 2048, 1024
f32, bf16, u32 = jnp.float32, jnp.bfloat16, jnp.uint32
T = 256
NB = S // T
H = T // 2
PITCH = 129
WROWS = 264
R2 = float(np.sqrt(0.5))
C8, S8 = float(np.cos(np.pi / 8)), float(np.sin(np.pi / 8))
SCALE = 2.0 / (S * D)


def _seeds():
    r = np.arange(8)[:, None]
    l = np.arange(128)[None, :]
    cls, j = l >> 6, l & 63
    tiles = []
    freqs = [8 * j, 8 * j + 4] + [8 * j + np.where(cls == 0, c, 8 - c) for c in (1, 2, 3)]
    for m in freqs:
        th, st = 2 * np.pi * r * m / D, 2 * np.pi * 8 * m / D + 0 * r
        tiles += [np.cos(th), np.sin(th), np.cos(st), np.sin(st)]
    for h in range(2):
        col = 128 * h + l
        b, odd = col >> 1, (col & 1) == 1
        al, st, tw = 2 * np.pi * r * b / 128, 2 * np.pi * 8 * b / 128 + 0 * r, 2 * np.pi * b / S + 0 * r
        tiles += [np.where(odd, np.sin(al), np.cos(al)), np.where(odd, np.cos(al), -np.sin(al)),
                  np.cos(st), np.sin(st), np.cos(tw), np.sin(tw)]
    tw = 2 * np.pi * r / S + 0 * l
    tiles += [np.cos(tw), np.sin(tw)]
    return np.stack(tiles).astype(np.float32)


def _iota(shape, axis):
    return jax.lax.broadcasted_iota(jnp.int32, shape, axis)


def _pack(a, b):
    return pltpu.pack_elementwise([a, b], packed_dtype=bf16)


def _unpack(w, i):
    return pltpu.unpack_elementwise(w, index=i, packed_dtype=bf16, unpacked_dtype=f32)


def _tiles(v):
    return [v[:, 128 * a:128 * (a + 1)] for a in range(v.shape[1] // 128)]


def _tree(op, xs):
    xs = list(xs)
    while len(xs) > 1:
        xs = [op(xs[i], xs[i + 1]) if i + 1 < len(xs) else xs[i] for i in range(0, len(xs), 2)]
    return xs[0]


def _rot(c, s, cs, ss):
    return c * cs - s * ss, s * cs + c * ss


def _layernorm(xs):
    m = jnp.sum(_tree(jnp.add, xs), axis=-1, keepdims=True) * (1.0 / D)
    xc = [x - m for x in xs]
    v = jnp.sum(_tree(jnp.add, [x * x for x in xc]), axis=-1, keepdims=True) * (1.0 / D)
    inv = jax.lax.rsqrt(v + 1e-5)
    return [x * inv for x in xc]


def _radix8_fwd(z):
    e = [z[a] + z[a + 4] for a in range(4)]
    o = [z[a] - z[a + 4] for a in range(4)]
    s02, s13 = e[0] + e[2], e[1] + e[3]
    p, q = (o[1] - o[3]) * R2, (o[1] + o[3]) * R2
    r1, n1, r2, i2, r3, i3 = o[0] + p, o[2] + q, e[0] - e[2], e[3] - e[1], o[0] - p, o[2] - q
    return [s02 + s13, s02 - s13, r1 - n1, r1, n1, r2 + i2, r2, i2, r3 + i3, r3, i3]


def _radix8_inv(t):
    t0, t4, r1, n1, r2, i2, r3, i3 = t
    a, b = t0 + t4, t0 - t4
    E = [a + r2, b - i2, a - r2, b + i2]
    u, v = r1 - r3, i3 - n1
    O = [r1 + r3, (u - v) * R2, i3 + n1, (u + v) * (-R2)]
    return [E[k] + O[k] for k in range(4)] + [E[k] - O[k] for k in range(4)]


def _dft4(x, sgn):
    (ar, ai), (br, bi), (cr, ci), (dr, di) = x
    sr, si, tr, ti = ar + cr, ai + ci, ar - cr, ai - ci
    ur, ui, vr, vi = br + dr, bi + di, br - dr, bi - di
    y1, y3 = (tr + vi, ti - vr), (tr - vi, ti + vr)
    if sgn > 0:
        y1, y3 = y3, y1
    return [(sr + ur, si + ui), y1, (sr - ur, si - ui), y3]


def _tw16(x, k, sgn):
    xr, xi = x
    k = k % 16
    if k == 0:
        return x
    if k == 4:
        return (xi, -xr) if sgn < 0 else (-xi, xr)
    if k == 2:
        return ((xr + xi) * R2, (xi - xr) * R2) if sgn < 0 else ((xr - xi) * R2, (xi + xr) * R2)
    if k == 6:
        return ((xi - xr) * R2, (xr + xi) * (-R2)) if sgn < 0 else ((xr + xi) * (-R2), (xr - xi) * R2)
    c, s = float(np.cos(np.pi * k / 8)), float(sgn * np.sin(np.pi * k / 8))
    return (xr * c - xi * s, xi * c + xr * s)


def _dft16(x, sgn):
    cols = [_dft4([x[a2 + 4 * a1] for a1 in range(4)], sgn) for a2 in range(4)]
    out = [None] * 16
    for k1 in range(4):
        y = _dft4([_tw16(cols[a2][k1], a2 * k1, sgn) for a2 in range(4)], sgn)
        for k2 in range(4):
            out[k1 + 4 * k2] = y[k2]
    return out


def _dot(a, b):
    return jnp.dot(a, b, preferred_element_type=f32)


def _dot_nt(a, b):
    return jax.lax.dot_general(a, b, (((1,), (1,)), ((), ())), preferred_element_type=f32)


def _b(w):
    return pltpu.bitcast(w, bf16)


def _w(v):
    return pltpu.bitcast(v.astype(bf16), u32)


def _strassen_lhs(top, bot):
    a11, a12 = jnp.concatenate(top[:4], axis=1), jnp.concatenate(top[4:], axis=1)
    a21, a22 = jnp.concatenate(bot[:4], axis=1), jnp.concatenate(bot[4:], axis=1)
    return [a11 + a22, a21 + a22, a11, a22, a11 + a12, a21 - a11, a12 - a22]


def _strassen_rhs(b11, b12, b21, b22):
    def comb(p, q, op):
        return _pack(op(_unpack(p, 0), _unpack(q, 0)), op(_unpack(p, 1), _unpack(q, 1)))
    return [comb(b11, b22, jnp.add), b11, comb(b12, b22, jnp.subtract), comb(b21, b11, jnp.subtract),
            b22, comb(b11, b12, jnp.add), comb(b21, b22, jnp.add)]


def _weave(never, mm, vec):
    def gate(tokens):
        def apply(v):
            if not tokens:
                return v
            t = v[0:8, 0:128]
            tok = _tree(jnp.bitwise_or, [k if k.dtype == u32 else pltpu.bitcast(k, u32) for k in tokens])
            t = jnp.where(never, tok if t.dtype == u32 else pltpu.bitcast(tok, t.dtype), t)
            if v.shape[1] > 128:
                t = jnp.concatenate([t, v[0:8, 128:]], axis=1)
            return jnp.concatenate([t, v[8:]], axis=0) if v.shape[0] > 8 else t
        return apply
    done, due = {}, {}
    for n in range(-1, len(mm)):
        if n >= 0:
            done[n] = mm[n](gate(due.pop(n, [])))
        for job, after, before in vec:
            if max(after, -1) == n:
                tied = before is not None
                tok = job(gate([done[n]] if tied and n >= 0 else []))
                if tied:
                    due.setdefault(before, []).append(tok[0:8, 0:128])


def _spread(jobs, lo, hi, window=None):
    out = []
    for k, job in enumerate(jobs):
        n = lo + (k * (hi - lo)) // len(jobs)
        out.append((job, n - 1, None if window is None else min(n + window, hi)))
    return out


def _cols(j, n=1):
    return pl.ds(128 * j, 128 * n)


def _kernel(x_hbm, wr_hbm, wi_hbm, wqkv_hbm, wo_hbm, seed_hbm, out_hbm,
            seed, xin, X, X2, Vp, U, dm, G, Gi, Wf, Wq, Wo, tb0, tb1, wr, wi, wq_raw, wo_raw, tmp, WE, sem):
    P_ = functools.partial
    sub = _iota((8, 128), 0)
    lane = _iota((8, 128), 1)
    lane16 = _iota((16, 128), 1)

    def x_copy(r0, i):
        return pltpu.make_async_copy(x_hbm.at[pl.ds(r0, T)], xin.at[pl.ds(r0, T)], sem.at[i])

    def out_copy(r0, i):
        return pltpu.make_async_copy(xin.at[pl.ds(r0, T)], out_hbm.at[pl.ds(r0, T)], sem.at[i])

    cp_seed = pltpu.make_async_copy(seed_hbm, seed, sem.at[NB])
    cp_w = [pltpu.make_async_copy(src, dst, sem.at[NB + 1 + q])
            for q, (src, dst) in enumerate(((wr_hbm, wr), (wi_hbm, wi)))]
    cp_q = [pltpu.make_async_copy(wqkv_hbm.at[:, pl.ds(D * n, D)], wq_raw.at[:, pl.ds(D * n, D)],
                                  sem.at[NB + 5 + n]) for n in range(3)]
    cp_o = pltpu.make_async_copy(wo_hbm, wo_raw, sem.at[NB + 8])
    cp_seed.start()
    x_copy(0, 0).start()
    x_copy(T, 1).start()
    cp_seed.wait()
    x_copy(2 * T, 2).start()

    zero = (seed[0] > 2.0).astype(jnp.int32)[0, 0]
    zero8 = pl.multiple_of(8 * zero, 8)
    regions = []

    def region(fn):
        regions.append(fn)
        pl.when(zero < len(regions))(fn)

    def weave(mm, vec):
        _weave(seed[0] > 2.0, mm, vec)

    def gen_dm():
        lo = lane16 < 64
        for n in range(5):
            c, s, cs, ss = (seed[4 * n + q] for q in range(4))
            for g in range(8):
                c2, s2 = _rot(c, s, cs, ss)
                cc, sc = jnp.concatenate([c, c2], axis=0), jnp.concatenate([s, s2], axis=0)
                rows = pl.ds(8 * g, 8)
                if n == 0:
                    alt = (1 - 2 * (_iota((16, 128), 0) & 1)).astype(f32)
                    dm[0, rows, :] = _w(jnp.where(lane16 == 64, alt, jnp.where(lo, cc, -sc)))
                elif n == 1:
                    dm[1, rows, :] = _w(jnp.where(lo, -sc, cc))
                else:
                    sc = jnp.where(lo, sc, -sc)
                    dm[3 * n - 4, rows, :] = _w(cc)
                    dm[3 * n - 3, rows, :] = _w(cc + sc)
                    dm[3 * n - 2, rows, :] = _w(cc - sc)
                if g < 7:
                    c, s = _rot(c2, s2, cs, ss)

    def gen_g(inverse):
        st = dict(pq=[seed[20], seed[21], seed[26], seed[27]], tw=(seed[32], seed[33]))
        c1, s1 = float(np.cos(2 * np.pi * 8 / S)), float(np.sin(2 * np.pi * 8 / S))

        def job(g, gate):
            rows, rows2 = pl.ds(8 * g, 8), pl.ds(64 + 8 * g, 8)
            tw1 = _rot(*st['tw'], c1, s1)
            cb, sb = (jnp.concatenate(v, axis=0) for v in zip(st['tw'], tw1))
            st['tw'] = _rot(*tw1, c1, s1)
            for h in range(2):
                p0, q0 = st['pq'][2 * h:2 * h + 2]
                cs, ss, ct, sn = (seed[22 + 6 * h + n] for n in range(4))
                q1, p1 = _rot(q0, p0, cs, ss)
                p, q = jnp.concatenate([p0, p1], axis=0), jnp.concatenate([q0, q1], axis=0)
                st['pq'][2 * h + 1], st['pq'][2 * h] = _rot(q1, p1, cs, ss)
                if inverse:
                    sg = (1 - 2 * (lane16 & 1)).astype(f32) * SCALE
                    p, q = p * sg, q * (-sg)
                    ct, sn = jnp.concatenate([ct, ct], axis=0), jnp.concatenate([sn, sn], axis=0)
                dst = Gi if inverse else G
                for a in range(16):
                    dst[a, rows, _cols(h)] = _w(p)
                    dst[a, rows2, _cols(h)] = _w(q)
                    if a < 15 and inverse:
                        p, q = _rot(p, q, ct, sn)
                    elif a < 15:
                        q, p = _rot(q, p, cb, sb)
        return [P_(job, g) for g in range(8)]

    def filter_tile(t, c, gate):
        we = WE.at[t]
        if c == 1:
            a = pltpu.bitcast(wr[0:512, _cols(t)], u32)
            b = pltpu.bitcast(wi[0:512, _cols(t)], u32)
            we[0:256] = (a & 0xFFFF) | (b << 16)
            we[256:512] = (a >> 16) | (b & jnp.uint32(0xFFFF0000))
        w = jnp.concatenate([we[pl.ds(256 * (r & 1) + (r >> 1), 64, stride=4), :]
                             for r in (c, (8 - c) if c else 4)], axis=0)
        if c == 0:
            def rows(src_t):
                return [jnp.broadcast_to(src[m:m + 1, _cols(src_t)].astype(f32), (8, 128))
                        for m in (0, D // 2) for src in (wr, wi)]
            ar, ai, br, bi = rows(t)
            cr, ci, dr, di = (jnp.take_along_axis(jnp.where(lane == 0, p, q), (128 - lane) & 127, axis=1)
                              for p, q in zip(rows((16 - t) % 16), rows(15 - t)))
            same = _pack(((ar + br) + (cr + dr)) * 0.125, ((ai + bi) - (ci + di)) * 0.125)
            pair = _pack(((ar - br) + (cr - dr)) * 0.125, ((ai - bi) - (ci - di)) * 0.125)
            w = jnp.concatenate([jnp.where(sub == 0, same, w[0:8]), w[8:]], axis=0)
            p = jnp.concatenate([jnp.where(sub == 0, pair, 0), jnp.zeros((120, 128), u32)], axis=0)
            Wf[4, pl.ds(128 * t, 128), :] = p.T
        Wf[c, pl.ds(128 * t, 128), :] = w.T

    x8 = lambda v: jnp.concatenate([v] * 8, axis=0)

    def spin_jobs(part):
        def spin(a, gate):
            l = lane
            src = x8(32 * ((l >> 2) & 3) + 16 * ((l >> 1) & 1) + 2 * (((l >> 4) - a) & 7) + (l & 1))
            for r in range(8):
                w = pltpu.bitcast(wq_raw[pl.ds(128 * r, 128), pl.ds(D * part + 128 * a, 128)], u32)
                tmp[part, a, pl.ds(64 * r, 64), :] = jnp.take_along_axis(w, src, axis=1)
        return [P_(spin, a) for a in range(8)]

    def gather_jobs(part):
        def gather(j, gate):
            l = lane
            rest = (((l >> 4) & 3) << 2) | ((l >> 6) << 1) | (l & 1)

            def col(jj, r0):
                v = tmp[part, 0, pl.ds(r0, 64), :]
                for a in range(1, 8):
                    v = jnp.where(x8(l >> 4) == ((jj + a) & 7), tmp[part, a, pl.ds(r0, 64), :], v)
                return jnp.take_along_axis(v, x8(((((l >> 1) + jj) & 7) << 4) | rest), axis=1)
            for r in range(4):
                b11, b21 = col(j, 64 * r), col(j, 256 + 64 * r)
                b12, b22 = col(j + 4, 64 * r), col(j + 4, 256 + 64 * r)
                for n, w in enumerate(_strassen_rhs(b11, b12, b21, b22)):
                    Wq[n, pl.ds(64 * r, 64), _cols(4 * part + j)] = w
        return [P_(gather, j) for j in range(4)]

    def wo_jobs():
        def stage(n, gate):
            w = pltpu.bitcast(wo_raw[:, _cols(n)], u32)
            for a in range(8):
                tmp[0, n, pl.ds(65 * a, 64), :] = w[64 * a:64 * a + 64]

        def gather(n, gate):
            for j in range(4):
                for g1 in range(2):
                    for b in range(4):
                        quad = [tmp[0, n + 4 * c, pl.ds(16 * b + 8 * g1 + j + 4 * r, 8, stride=65), :]
                                for r in range(2) for c in range(2)]
                        for q, w in enumerate(_strassen_rhs(*quad)):
                            Wo[q, pl.ds(64 * j + 32 * g1 + 8 * b, 8), _cols(n)] = w
        return [P_(stage, n) for n in range(8)] + [P_(gather, n) for n in range(4)]

    def ln_radix8(tb, g, xs):
        w = _w(jnp.concatenate(_radix8_fwd(_layernorm(xs)), axis=1))
        tb[pl.ds(8 * g, 8), :] = w
        return w

    def dft_d(r0, tb, c, gate):
        lo = _iota((T, 128), 1) < 64
        if c == 0:
            a = _dot(_b(tb[:, 0:128]), _b(gate(dm[0])))
            b = _dot(_b(tb[:, 128:256]), _b(dm[1]))
            w = _pack(jnp.where(lo, a, b), pltpu.roll(jnp.where(lo, b, a), 64, 1))
        else:
            ys, yr, yi = (_dot(_b(tb[:, _cols(n)]), _b(dm[n])) for n in range(3 * c - 1, 3 * c + 2))
            w = _pack(ys + yi if c == 1 else ys - yi, (ys - yr) * jnp.where(lo, 1.0, -1.0))
        for g in range(T // 8):
            Vp[c, pl.ds((g % 2) * 8 * PITCH + r0 // 16 + g // 2, 8, stride=PITCH), :] = w[8 * g:8 * g + 8, :]
        return w[0:8]

    def spectral(first, *R):
        def mm1(c, a, gate):
            v = Vp[c, pl.ds(a * PITCH, 128), :]
            if c == 0:
                R[c][a, 0:256, :] = _dot(_b(G[a]), _b(v))
            else:
                for h in range(2):
                    R[c][a, pl.ds(256 * h, 256), :] = _dot(_b(G[a, :, _cols(h)]), _b(v[64 * h:64 * h + 64]))

        def mid(c, g, gate):
            def load(a, r):
                v = R[c][a, pl.ds(r, 8), :]
                return v + R[c][a, pl.ds(256 + r, 8), :] if c else v
            y = _dft16([(load(a, 8 * g), load(a, 128 + 8 * g)) for a in range(16)], -1)
            if c == 0:
                part = []
                for a in range(16):
                    if g:
                        part.append(tuple(jnp.take_along_axis(load(a, o + 121 - 8 * g), 7 - sub, axis=0)
                                          for o in (0, 128)))
                    else:
                        w0 = _tw16((load(a, 0), load(a, 128)), a, -1)
                        part.append(tuple(
                            jnp.take_along_axis(jnp.where(sub == 0, p, load(a, o + 120)), (8 - sub) & 7, axis=0)
                            for p, o in zip(w0, (0, 128))))
                yneg = _dft16(part, -1)
            z = []
            for k1 in range(16):
                yr, yi = y[k1]
                w = Wf[c, pl.ds(128 * k1 + 8 * g, 8), :]
                ar, ai = _unpack(w, 0), _unpack(w, 1)
                zr, zi = yr * ar - yi * ai, yr * ai + yi * ar
                if c == 0:
                    w = Wf[4, pl.ds(128 * k1 + 8 * g, 8), :]
                    br, bi = _unpack(w, 0), _unpack(w, 1)
                    pr, pi = yneg[15 - k1]
                    zr, zi = zr + (pr * br + pi * bi), zi + (pr * bi - pi * br)
                z.append((zr, zi))
            for a, v in enumerate(_dft16(z, 1)):
                w = pltpu.bitcast(_pack(*v), f32)
                R[c][a, pl.ds(zero8 + 512 + 8 * g, 8), :] = w
            if g == 15 and c < 3 and not first:
                R[c + 1][0, pl.ds(zero8 + 640, 8), :] = w

        def mm2(c, a, gate):
            v = pltpu.bitcast(R[c][a, 512:640, :], u32)
            for h in range(2):
                u = _dot(_b(Gi[a, :, _cols(h)]), _b(v[64 * h:64 * h + 64]))
                U[2 * h, c, pl.ds(a * PITCH, 128), :] = u[:128]
                U[2 * h + 1, c, pl.ds(a * PITCH, 128), :] = u[128:]

        m1 = lambda c: [P_(mm1, c, a) for a in range(16)]
        m2 = lambda c: [P_(mm2, c, a) for a in range(16)]
        mids = lambda c: [P_(mid, c, g) for g in range(16)]

        def run(mm, vec, before=None):
            def fn():
                if before:
                    before()
                weave(mm, _spread(vec() if callable(vec) else vec, 0, len(mm)))
            region(fn)

        if first:
            def wait(*cps):
                return lambda: [cp.wait() for cp in cps]

            def merge(p, q):
                order = sorted([(n / len(p), 0, n) for n in range(len(p))]
                               + [((n + 0.5) / len(q), 1, n) for n in range(len(q))])
                return [(p, q)[src][n] for _, src, n in order]
            filt = lambda c: [P_(filter_tile, t, c) for t in range(16)]
            run(m1(0) + m1(1), lambda: gen_g(True))
            run(m1(2), filt(1), lambda: (wait(*cp_w)(), cp_q[0].start(), cp_q[1].start()))
            run(m1(3), merge(mids(1), filt(2) + filt(0)[:4]))
            run(m2(1), merge(mids(2), filt(3) + filt(0)[4:8]), lambda: (cp_q[2].start(), cp_o.start()))
            run(m2(2), merge(mids(3), filt(0)[8:]))
            run(m2(3), merge(mids(0), spin_jobs(0)), wait(cp_q[0]))
            run(m2(0), merge(gather_jobs(0), spin_jobs(1)), wait(cp_q[1]))
        else:
            run(m1(0), [])
            v = mids(0) + mids(1) + mids(2) + mids(3)
            c0, c1, c2 = map(int, '16,42,53'.split(','))
            run(m1(1) + m1(2), v[:c0])
            run(m1(3) + m2(0), v[c0:c1])
            run(m2(1), v[c1:c2])
            run(m2(2), v[c2:])
            run(m2(3), [])

    def run_spectral(first):
        pl.run_scoped(P_(spectral, first), *[pltpu.VMEM((16, 648, 128), f32)] * 4)

    def rowwise(last, ub, ya, yb, zf, o0, o1, z0, z1, QK0, QK1, VO0, VO1):
        bufs = ((QK0, VO0), (QK1, VO1))

        def idft_operands(r0, c, gate):
            def get(q):
                return jnp.concatenate(
                    [U[q, c, pl.ds(r0 // 16 + g, 16, stride=PITCH), :]
                     + U[q + 2, c, pl.ds(r0 // 16 + g, 16, stride=PITCH), :] for g in range(T // 16)], axis=0)
            lo = _iota((T, 128), 1) < 64
            ur, ui = gate(get(0)), get(1)
            if c == 0:
                ui = pltpu.roll(ui, 64, 1)
                ops = jnp.where(lo, ur, ui), jnp.where(lo, ui, ur)
            else:
                ui = ui * jnp.where(lo, 1.0, -1.0)
                ops = ur + ui, ui, ur
            for n, u in enumerate(ops):
                w = _w(u)
                ub[:, _cols(max(3 * c - 1, 0) + n)] = w
            return w[-8:]

        def idft_d(ya, c, gate):
            if c == 0:
                ya[:, 0:128] = _dot_nt(_b(ub[:, 0:128]), _b(gate(dm[0])))
                y = _dot_nt(_b(ub[:, 128:256]), _b(dm[1]))
            else:
                ys, yi, yr = (_dot_nt(_b(ub[:, _cols(n)]), _b(dm[n])) for n in range(3 * c - 1, 3 * c + 2))
                ya[:, _cols(2 * c)] = ys - yi
                y = yr - ys if c == 1 else ys - yr
            ya[:, _cols(2 * c + 1)] = y
            return y[0:8]

        def ln_attn(r0, ya, g, gate):
            rr, rows = pl.ds(r0 + 16 * g, 16), pl.ds(16 * g, 16)
            yt = _tiles(ya[rows, :])
            yt[0] = gate(yt[0])
            x0 = X2[rr, :] if last else xin[rr, :].astype(f32)
            xs = [a + b for a, b in zip(_tiles(x0), _radix8_inv(yt))]
            X[rr, :] = jnp.concatenate(xs, axis=1)
            z = jnp.concatenate(_layernorm(xs), axis=1)
            zf[rows, :] = z
            return z

        def operands(get, dst, g, gate):
            top, bot = get(pl.ds(16 * g, 16)), get(pl.ds(H + 16 * g, 16))
            top[0] = gate(top[0])
            for q, a in enumerate(_strassen_lhs(top, bot)):
                w = _w(a)
                dst[q, pl.ds(8 * g, 8), :] = w
            return w

        def strassen(A, B, n, put):
            m = {}

            def mm(q, gate=lambda v: v):
                return _dot(_b(A[q]), _b(gate(B[q, :, _cols(n)])))

            def j1(gate):
                m[1], m[2] = mm(0, gate), mm(1)
                return m[2][0:8]

            def j2(gate):
                m[3] = mm(2, gate)
                c22 = ((m[1] - m[2]) + m[3]) + mm(5)
                put(1, 1, c22)
                return c22[0:8]

            def j3(gate):
                m4 = mm(3, gate)
                put(1, 0, m[2] + m4)
                m5 = mm(4)
                put(0, 1, m[3] + m5)
                m[1] = (m[1] + m4) - m5
                return m5[0:8]

            def j4(gate):
                c11 = m[1] + mm(6, gate)
                put(0, 0, c11)
                return c11[0:8]
            if 1 == 3:
                return [j1, j2, j3, j4]
            return [lambda gate: (j1(gate), j2(lambda v: v))[1], lambda gate: (j3(gate), j4(lambda v: v))[1]]

        def proj(z, par, n):
            part = n // 4
            dst, t0 = bufs[par][part >> 1], 8 * (part & 1)

            def put(r, c, y):
                dst[t0 + 4 * c + n % 4, pl.ds(16 + r * H, H), :] = y
            return strassen(z, Wq, n, put)

        def softmax(r0, par, rr, gate):
            QK = bufs[par][0]
            q = [QK[j, pl.ds(16 + rr, 8), :] for j in range(8)]
            q[0] = gate(q[0])
            L = []
            for w in range(8):
                p = _tree(jnp.add, [q[j] * QK[8 + j, pl.ds(16 + rr - 2 * w, 8), :] for j in range(8)])
                p = p + pltpu.roll(p, 64, 1)
                p = p + jnp.take_along_axis(p, lane ^ 1, axis=1)
                if rr < 2 * w:
                    p = jnp.where(r0 + rr + sub >= 2 * w, p, -1e9 * 32 ** 0.5)
                L.append(p)
            m = _tree(jnp.maximum, L)
            e = [jnp.exp2((l - m) * float(32 ** -0.5 * np.log2(np.e))) for l in L]
            inv = 1.0 / _tree(jnp.add, e)
            return [v * inv for v in e]

        def mix(par, rr, z8, p):
            VO = bufs[par][1]
            for j in range(8):
                o = _tree(jnp.add, [p[w] * VO[j, pl.ds(16 + rr - 2 * w, 8), :] for w in range(8)])
                VO[8 + j, pl.ds(z8 + rr, 8), :] = o
            return o

        def attend(r0, par, rr, ordered, gate):
            p = softmax(r0, par, rr, gate)
            if ordered:
                QK = bufs[par][0]
                for w in range(8):
                    QK[16 + w, pl.ds(zero8 + rr, 8), :] = p[w]
                p = [QK[16 + w, pl.ds(rr, 8), :] for w in range(8)]
            return mix(par, rr, zero8 if ordered else 0, p)

        def out_proj(r0, ob, yb, n):
            def put(r, c, y):
                at = (pl.ds(r0 + r * H, H), _cols(4 * c + n))
                if last:
                    xin[at] = (X[at] + y).astype(bf16)
                else:
                    yb[pl.ds(r * H, H), _cols(4 * c + n)] = X[at] + y
            return strassen(ob, Wo, n, put)

        def residual(r0, tb, yb, g, gate):
            v = gate(yb[pl.ds(16 * g, 16), :])
            X2[pl.ds(r0 + 16 * g, 16), :] = v
            return ln_radix8(tb, g, _tiles(v))

        def fourfold(fn):
            def job(cs, gate):
                return [fn(c, gate if c == cs[0] else (lambda v: v)) for c in cs][-1]
            return [P_(job, (0, 1)), P_(job, (2, 3))] if 1 == 1 else [P_(job, (c,)) for c in range(4)]
        m_idft = lambda y=ya: fourfold(P_(idft_d, y))
        v_iop = lambda r0: [P_(idft_operands, r0, c) for c in range(4)]
        m_proj = lambda par, lo=0, hi=12: [j for n in range(lo, hi) for j in proj((z0, z1)[par], par, n)]
        m_out = lambda r0, ob, y=yb: [j for n in range(4) for j in out_proj(r0, ob, y, n)]
        m_dft = lambda r0, tb=tb0: [] if last else fourfold(P_(dft_d, r0, tb))

        def v_ln(r0, par, y=ya):
            jobs = []
            for g in range(H // 16):
                jobs += [P_(ln_attn, r0, y, g), P_(ln_attn, r0, y, g + H // 16),
                         P_(operands, lambda rows: _tiles(zf[rows, :]), (z0, z1)[par], g)]
            return jobs

        def v_att(r0, par, ordered=True, dst=None):
            jobs = []
            for g in range(H // 16):
                jobs += [P_(attend, r0, par, h + 16 * g + e, ordered) for h in (0, H) for e in (0, 8)]
                jobs += [P_(operands, lambda rows: [bufs[par][1][8 + j, rows, :] for j in range(8)],
                            (o0, o1)[par] if dst is None else dst, g)]
            return jobs
        v_res = lambda r0, tb=tb0, y=yb: [] if last else [P_(residual, r0, tb, y, g) for g in range(T // 16)]

        def halo(par, first=False):
            for j in range(8):
                for dst, src, t in zip(bufs[par], bufs[1 - par], (8 + j, j)):
                    dst[t, 0:16, :] = jnp.zeros((16, 128), f32) if first else src[t, T:T + 16, :]

        def head0():
            halo(0, True)
            weave(m_idft(yb) + m_idft(),
                  _spread(v_iop(0), 0, 0) + _spread(v_iop(T), 2, 2) + _spread(v_ln(0, 0, yb), 2, 4))

        def head(part):
            if part < 2:
                (cp_q[2], cp_o)[part].wait()
            vec = (_spread(gather_jobs(1), 0, 8) + _spread(spin_jobs(2), 0, 8),
                   _spread(gather_jobs(2), 0, 8) + _spread(wo_jobs()[:8], 0, 8),
                   _spread(wo_jobs()[8:], 0, 8))[part]
            weave(m_proj(0, 4 * part, 4 * part + 4), vec + _spread(v_ln(T, 1)[8 * part:8 * part + 8], 0, 8))

        def step(i, par, nxt=True, old=True):
            rn, rp, ro = ((i + d) * T if isinstance(i, int) else pl.multiple_of((i + d) * T, T) for d in (1, -1, -2))
            halo(par)
            mo, mi = m_out(ro, (o0, o1)[par]) if old else [], m_idft() if nxt else []
            a, b, f = len(mo), len(mo) + len(mi), 1 + 1
            na, nl, wl = (11, 11, 2) if last else (13, 13, 2)
            cut = 0
            if not old:
                na, nl = 11, 11
            vec = _spread(v_att(rp, 1 - par), 0, b + f * na, 4 if old else 3)
            if old:
                vec += _spread(v_res(ro), a + f * 0, b + f * 11, 2)
            if nxt:
                vec += _spread(v_iop(rn), 0, a, 2 if old else None)
                vec += _spread(v_ln(rn, 1 - par), b, b + f * (nl - cut), 2 if last else wl)
            p, md = m_proj(par), m_dft(ro) if old else []
            k = f * min(12, 11)
            weave(mo + mi + p[:k] + md + p[k:], vec)
            if last and old:
                out_copy(ro, i - 2).start()

        r5, r6, r7 = ((NB - d) * T for d in (3, 2, 1))

        def tail0():
            halo(1)
            weave(m_proj(1), _spread(v_att(r6, 0), 0, 22, 4))

        def tail1():
            weave(m_out(r5, o1, ya) + m_out(r6, o0) + m_dft(r5),
                  _spread(v_att(r7, 1, False, z0), 0, 14, 4) + _spread(v_res(r5, tb0, ya), 8, 16, 2))
            if last:
                out_copy(r5, NB - 3).start()
                out_copy(r6, NB - 2).start()

        def tail2():
            weave(m_out(r7, z0, ya) + m_dft(r6), _spread(v_res(r6), 0, 7, 2))
            if last:
                out_copy(r7, NB - 1).start()
            for job in v_res(r7, tb1, ya):
                job(lambda v: v)
            weave(m_dft(r7, tb1), [])

        def head_all():
            weave(m_proj(0), _spread(v_ln(T, 1), 0, 22, 2))
        heads = [head_all] if last else [P_(head, part) for part in range(3)]
        for fn in [head0] + heads + [P_(step, 1, 1, True, False)]:
            region(fn)

        def loop(i, _):
            for par in range(2):
                pl.when(i % 2 == par)(P_(step, i, par))
            return _
        jax.lax.fori_loop(2, NB - 1, loop, 0)
        for fn in (tail0, tail1, tail2):
            region(fn)

    def run_rowwise(last):
        zs = pltpu.VMEM((7, H // 2, 512), u32)
        rows, qk, vo = pltpu.VMEM((T, D), f32), pltpu.VMEM((24, 16 + T, 128), f32), pltpu.VMEM((16, 16 + T, 128), f32)
        pl.run_scoped(P_(rowwise, last), pltpu.VMEM((T // 2, 11 * 128), u32), rows, rows, rows, zs, zs, zs, zs, qk, qk, vo, vo)

    gen_dm()

    def ln_x(r0, tb, g, gate):
        return ln_radix8(tb, g, _tiles(xin[pl.ds(r0 + 16 * g, 16), :].astype(f32)))

    def first_dft(i, par):
        r0 = pl.multiple_of(i * T, T)
        x_copy(r0, i).wait()

        @pl.when(i + 3 < NB)
        def _():
            x_copy(pl.multiple_of(jnp.minimum(i + 3, NB - 1) * T, T), jnp.minimum(i + 3, NB - 1)).start()

        @pl.when(i + 3 == NB)
        def _():
            for cp in cp_w:
                cp.start()
        weave([P_(dft_d, r0 - T, (tb0, tb1)[1 - par], c) for c in range(4)],
              _spread([P_(ln_x, r0, (tb0, tb1)[par], g) for g in range(T // 16)], 0, 4, 2))

    def first_ln():
        x_copy(0, 0).wait()
        x_copy(3 * T, 3).start()
        weave([], _spread([P_(ln_x, 0, tb0, g) for g in range(T // 16)], 0, 0))

    def first_loop(i, _):
        for par in range(2):
            pl.when(i % 2 == par)(P_(first_dft, i, par))
        return _

    region(first_ln)
    jax.lax.fori_loop(1, NB, first_loop, 0)
    region(lambda: weave([P_(dft_d, (NB - 1) * T, tb1, c) for c in range(4)], _spread(gen_g(False), 0, 4)))
    run_spectral(True)
    run_rowwise(False)
    run_spectral(False)
    run_rowwise(True)
    for i in range(NB):
        out_copy(i * T, i).wait()


@jax.jit
def pallas_interleave_layers__spectral_gfnet__sliding_local_dilated__prompt_kernel(A_x, A_w_r, A_w_i, B_x, B_wqkv, B_wo):
    del B_x
    hbm = pl.BlockSpec(memory_space=pltpu.HBM)
    args = (A_x.reshape(S, D), A_w_r.T, A_w_i.T, B_wqkv, B_wo, jnp.asarray(_seeds()))
    out = pl.pallas_call(
        _kernel,
        out_shape=jax.ShapeDtypeStruct((S, D), bf16),
        in_specs=[hbm] * 6,
        out_specs=hbm,
        scratch_shapes=[
            pltpu.VMEM((34, 8, 128), f32),
            pltpu.VMEM((S, D), bf16),
            pltpu.VMEM((S, D), f32),
            pltpu.VMEM((S, D), f32),
            pltpu.VMEM((4, 17 * PITCH - 1, 128), u32),
            pltpu.VMEM((4, 4, 17 * PITCH - 1, 128), f32),
            pltpu.VMEM((11, 64, 128), u32),
            pltpu.VMEM((16, 128, 256), u32),
            pltpu.VMEM((16, 128, 256), u32),
            pltpu.VMEM((5, S, 128), u32),
            pltpu.VMEM((7, 256, 1536), u32),
            pltpu.VMEM((7, 256, 512), u32),
            pltpu.VMEM((T // 2, 11 * 128), u32),
            pltpu.VMEM((T // 2, 11 * 128), u32),
            pltpu.VMEM((513, S), bf16),
            pltpu.VMEM((513, S), bf16),
            pltpu.VMEM((D, 3 * D), bf16),
            pltpu.VMEM((D, D), bf16),
            pltpu.VMEM((3, 8, 584, 128), u32),
            pltpu.VMEM((16, 520, 128), u32),
            pltpu.SemaphoreType.DMA((NB + 9,)),
        ],
        compiler_params=pltpu.CompilerParams(vmem_limit_bytes=127 * 1024 * 1024),
    )(*args)
    return out.reshape(1, S, D)
```

```python
import functools
import numpy as np
import jax
import jax.numpy as jnp
from jax.experimental import pallas as pl
from jax.experimental.pallas import tpu as pltpu

S, D = 2048, 1024
f32, bf16, u32 = jnp.float32, jnp.bfloat16, jnp.uint32
T = 256
NB = S // T
H = T // 2
PITCH = 129
R2 = float(np.sqrt(0.5))
SCALE = 2.0 / (S * D)


def _seeds():
    r = np.arange(8)[:, None]
    l = np.arange(128)[None, :]
    cls, j = l >> 6, l & 63
    tiles = []
    freqs = [8 * j, 8 * j + 4] + [8 * j + np.where(cls == 0, c, 8 - c) for c in (1, 2, 3)]
    for m in freqs:
        th, st = 2 * np.pi * r * m / D, 2 * np.pi * 8 * m / D + 0 * r
        tiles += [np.cos(th), np.sin(th), np.cos(st), np.sin(st)]
    for h in range(2):
        col = 128 * h + l
        b, odd = col >> 1, (col & 1) == 1
        al, st, tw = 2 * np.pi * r * b / 128, 2 * np.pi * 8 * b / 128 + 0 * r, 2 * np.pi * b / S + 0 * r
        tiles += [np.where(odd, np.sin(al), np.cos(al)), np.where(odd, np.cos(al), -np.sin(al)),
                  np.cos(st), np.sin(st), np.cos(tw), np.sin(tw)]
    tw = 2 * np.pi * r / S + 0 * l
    tiles += [np.cos(tw), np.sin(tw)]
    return np.stack(tiles).astype(np.float32)


def _iota(shape, axis):
    return jax.lax.broadcasted_iota(jnp.int32, shape, axis)


def _pack(a, b):
    return pltpu.pack_elementwise([a, b], packed_dtype=bf16)


def _unpack(w, i):
    return pltpu.unpack_elementwise(w, index=i, packed_dtype=bf16, unpacked_dtype=f32)


def _tiles(v):
    return [v[:, 128 * a:128 * (a + 1)] for a in range(v.shape[1] // 128)]


def _tree(op, xs):
    xs = list(xs)
    while len(xs) > 1:
        xs = [op(xs[i], xs[i + 1]) if i + 1 < len(xs) else xs[i] for i in range(0, len(xs), 2)]
    return xs[0]


def _rot(c, s, cs, ss):
    return c * cs - s * ss, s * cs + c * ss


def _layernorm(xs):
    m = jnp.sum(_tree(jnp.add, xs), axis=-1, keepdims=True) * (1.0 / D)
    xc = [x - m for x in xs]
    v = jnp.sum(_tree(jnp.add, [x * x for x in xc]), axis=-1, keepdims=True) * (1.0 / D)
    inv = jax.lax.rsqrt(v + 1e-5)
    return [x * inv for x in xc]


def _radix8_fwd(z):
    e = [z[a] + z[a + 4] for a in range(4)]
    o = [z[a] - z[a + 4] for a in range(4)]
    s02, s13 = e[0] + e[2], e[1] + e[3]
    p, q = (o[1] - o[3]) * R2, (o[1] + o[3]) * R2
    r1, n1, r2, i2, r3, i3 = o[0] + p, o[2] + q, e[0] - e[2], e[3] - e[1], o[0] - p, o[2] - q
    return [s02 + s13, s02 - s13, r1 - n1, r1, n1, r2 + i2, r2, i2, r3 + i3, r3, i3]


def _radix8_inv(t):
    t0, t4, r1, n1, r2, i2, r3, i3 = t
    a, b = t0 + t4, t0 - t4
    E = [a + r2, b - i2, a - r2, b + i2]
    u, v = r1 - r3, i3 - n1
    O = [r1 + r3, (u - v) * R2, i3 + n1, (u + v) * (-R2)]
    return [E[k] + O[k] for k in range(4)] + [E[k] - O[k] for k in range(4)]


def _dft4(x, sgn):
    (ar, ai), (br, bi), (cr, ci), (dr, di) = x
    sr, si, tr, ti = ar + cr, ai + ci, ar - cr, ai - ci
    ur, ui, vr, vi = br + dr, bi + di, br - dr, bi - di
    y1, y3 = (tr + vi, ti - vr), (tr - vi, ti + vr)
    if sgn > 0:
        y1, y3 = y3, y1
    return [(sr + ur, si + ui), y1, (sr - ur, si - ui), y3]


def _tw16(x, k, sgn):
    xr, xi = x
    k = k % 16
    if k == 0:
        return x
    if k == 4:
        return (xi, -xr) if sgn < 0 else (-xi, xr)
    if k == 2:
        return ((xr + xi) * R2, (xi - xr) * R2) if sgn < 0 else ((xr - xi) * R2, (xi + xr) * R2)
    if k == 6:
        return ((xi - xr) * R2, (xr + xi) * (-R2)) if sgn < 0 else ((xr + xi) * (-R2), (xr - xi) * R2)
    c, s = float(np.cos(np.pi * k / 8)), float(sgn * np.sin(np.pi * k / 8))
    return (xr * c - xi * s, xi * c + xr * s)


def _dft16(x, sgn):
    cols = [_dft4([x[a2 + 4 * a1] for a1 in range(4)], sgn) for a2 in range(4)]
    out = [None] * 16
    for k1 in range(4):
        y = _dft4([_tw16(cols[a2][k1], a2 * k1, sgn) for a2 in range(4)], sgn)
        for k2 in range(4):
            out[k1 + 4 * k2] = y[k2]
    return out


def _dot(a, b):
    return jnp.dot(a, b, preferred_element_type=f32)


def _dot_nt(a, b):
    return jax.lax.dot_general(a, b, (((1,), (1,)), ((), ())), preferred_element_type=f32)


def _b(w):
    return pltpu.bitcast(w, bf16)


def _w(v):
    return pltpu.bitcast(v.astype(bf16), u32)


def _strassen_lhs(top, bot):
    a11, a12 = jnp.concatenate(top[:4], axis=1), jnp.concatenate(top[4:], axis=1)
    a21, a22 = jnp.concatenate(bot[:4], axis=1), jnp.concatenate(bot[4:], axis=1)
    return [a11 + a22, a21 + a22, a11, a22, a11 + a12, a21 - a11, a12 - a22]


def _strassen_rhs(b11, b12, b21, b22):
    def comb(p, q, op):
        return _pack(op(_unpack(p, 0), _unpack(q, 0)), op(_unpack(p, 1), _unpack(q, 1)))
    return [comb(b11, b22, jnp.add), b11, comb(b12, b22, jnp.subtract), comb(b21, b11, jnp.subtract),
            b22, comb(b11, b12, jnp.add), comb(b21, b22, jnp.add)]


def _weave(never, mm, vec):
    def gate(tokens):
        def apply(v):
            if not tokens:
                return v
            t = v[0:8, 0:128]
            tok = _tree(jnp.bitwise_or, [k if k.dtype == u32 else pltpu.bitcast(k, u32) for k in tokens])
            t = jnp.where(never, tok if t.dtype == u32 else pltpu.bitcast(tok, t.dtype), t)
            if v.shape[1] > 128:
                t = jnp.concatenate([t, v[0:8, 128:]], axis=1)
            return jnp.concatenate([t, v[8:]], axis=0) if v.shape[0] > 8 else t
        return apply
    done, due = {}, {}
    for n in range(-1, len(mm)):
        if n >= 0:
            done[n] = mm[n](gate(due.pop(n, [])))
        for job, after, before in vec:
            if max(after, -1) == n:
                tied = before is not None
                tok = job(gate([done[n]] if tied and n >= 0 else []))
                if tied:
                    due.setdefault(before, []).append(tok[0:8, 0:128])


def _spread(jobs, lo, hi, window=None):
    out = []
    for k, job in enumerate(jobs):
        n = lo + (k * (hi - lo)) // len(jobs)
        out.append((job, n - 1, None if window is None else min(n + window, hi)))
    return out


def _cols(j, n=1):
    return pl.ds(128 * j, 128 * n)


def _kernel(x_hbm, wr_hbm, wi_hbm, wqkv_hbm, wo_hbm, seed_hbm, out_hbm,
            seed, xin, X, X2, Vp, U, dm, G, Gi, Wf, Wq, Wo, tb0, tb1, wr, wi, wq_raw, wo_raw, tmp, WE, sem):
    P_ = functools.partial
    sub = _iota((8, 128), 0)
    lane = _iota((8, 128), 1)
    lane16 = _iota((16, 128), 1)

    def x_copy(r0, i):
        return pltpu.make_async_copy(x_hbm.at[pl.ds(r0, T)], xin.at[pl.ds(r0, T)], sem.at[i])

    def out_copy(r0, i):
        return pltpu.make_async_copy(xin.at[pl.ds(r0, T)], out_hbm.at[pl.ds(r0, T)], sem.at[i])

    cp_seed = pltpu.make_async_copy(seed_hbm, seed, sem.at[NB])
    cp_w = [pltpu.make_async_copy(src, dst, sem.at[NB + 1 + q])
            for q, (src, dst) in enumerate(((wr_hbm, wr), (wi_hbm, wi)))]
    cp_q = [pltpu.make_async_copy(wqkv_hbm.at[:, pl.ds(D * n, D)], wq_raw.at[:, pl.ds(D * n, D)],
                                  sem.at[NB + 5 + n]) for n in range(3)]
    cp_o = pltpu.make_async_copy(wo_hbm, wo_raw, sem.at[NB + 8])
    cp_seed.start()
    x_copy(0, 0).start()
    x_copy(T, 1).start()
    cp_seed.wait()
    x_copy(2 * T, 2).start()

    zero = (seed[0] > 2.0).astype(jnp.int32)[0, 0]
    zero8 = pl.multiple_of(8 * zero, 8)
    regions = []

    def region(fn):
        regions.append(fn)
        pl.when(zero < len(regions))(fn)

    def weave(mm, vec):
        _weave(seed[0] > 2.0, mm, vec)

    def gen_dm():
        lo = lane16 < 64
        for n in range(5):
            c, s, cs, ss = (seed[4 * n + q] for q in range(4))
            for g in range(8):
                c2, s2 = _rot(c, s, cs, ss)
                cc, sc = jnp.concatenate([c, c2], axis=0), jnp.concatenate([s, s2], axis=0)
                rows = pl.ds(8 * g, 8)
                if n == 0:
                    alt = (1 - 2 * (_iota((16, 128), 0) & 1)).astype(f32)
                    dm[0, rows, :] = _w(jnp.where(lane16 == 64, alt, jnp.where(lo, cc, -sc)))
                elif n == 1:
                    dm[1, rows, :] = _w(jnp.where(lo, -sc, cc))
                else:
                    sc = jnp.where(lo, sc, -sc)
                    dm[3 * n - 4, rows, :] = _w(cc)
                    dm[3 * n - 3, rows, :] = _w(cc + sc)
                    dm[3 * n - 2, rows, :] = _w(cc - sc)
                if g < 7:
                    c, s = _rot(c2, s2, cs, ss)

    def gen_g(inverse):
        st = dict(pq=[seed[20], seed[21], seed[26], seed[27]], tw=(seed[32], seed[33]))
        c1, s1 = float(np.cos(2 * np.pi * 8 / S)), float(np.sin(2 * np.pi * 8 / S))

        def job(g, gate):
            rows, rows2 = pl.ds(8 * g, 8), pl.ds(64 + 8 * g, 8)
            tw1 = _rot(*st['tw'], c1, s1)
            cb, sb = (jnp.concatenate(v, axis=0) for v in zip(st['tw'], tw1))
            st['tw'] = _rot(*tw1, c1, s1)
            for h in range(2):
                p0, q0 = st['pq'][2 * h:2 * h + 2]
                cs, ss, ct, sn = (seed[22 + 6 * h + n] for n in range(4))
                q1, p1 = _rot(q0, p0, cs, ss)
                p, q = jnp.concatenate([p0, p1], axis=0), jnp.concatenate([q0, q1], axis=0)
                st['pq'][2 * h + 1], st['pq'][2 * h] = _rot(q1, p1, cs, ss)
                if inverse:
                    sg = (1 - 2 * (lane16 & 1)).astype(f32) * SCALE
                    p, q = p * sg, q * (-sg)
                    ct, sn = jnp.concatenate([ct, ct], axis=0), jnp.concatenate([sn, sn], axis=0)
                dst = Gi if inverse else G
                for a in range(16):
                    dst[a, rows, _cols(h)] = _w(p)
                    dst[a, rows2, _cols(h)] = _w(q)
                    if a < 15 and inverse:
                        p, q = _rot(p, q, ct, sn)
                    elif a < 15:
                        q, p = _rot(q, p, cb, sb)
        return [P_(job, g) for g in range(8)]

    def filter_tile(t, c, gate):
        we = WE.at[t]
        if c == 1:
            a = pltpu.bitcast(wr[0:512, _cols(t)], u32)
            b = pltpu.bitcast(wi[0:512, _cols(t)], u32)
            we[0:256] = (a & 0xFFFF) | (b << 16)
            we[256:512] = (a >> 16) | (b & jnp.uint32(0xFFFF0000))
        w = jnp.concatenate([we[pl.ds(256 * (r & 1) + (r >> 1), 64, stride=4), :]
                             for r in (c, (8 - c) if c else 4)], axis=0)
        if c == 0:
            def rows(src_t):
                return [jnp.broadcast_to(src[m:m + 1, _cols(src_t)].astype(f32), (8, 128))
                        for m in (0, D // 2) for src in (wr, wi)]
            ar, ai, br, bi = rows(t)
            cr, ci, dr, di = (jnp.take_along_axis(jnp.where(lane == 0, p, q), (128 - lane) & 127, axis=1)
                              for p, q in zip(rows((16 - t) % 16), rows(15 - t)))
            same = _pack(((ar + br) + (cr + dr)) * 0.125, ((ai + bi) - (ci + di)) * 0.125)
            pair = _pack(((ar - br) + (cr - dr)) * 0.125, ((ai - bi) - (ci - di)) * 0.125)
            w = jnp.concatenate([jnp.where(sub == 0, same, w[0:8]), w[8:]], axis=0)
            p = jnp.concatenate([jnp.where(sub == 0, pair, 0), jnp.zeros((120, 128), u32)], axis=0)
            Wf[4, pl.ds(128 * t, 128), :] = p.T
        Wf[c, pl.ds(128 * t, 128), :] = w.T

    x8 = lambda v: jnp.concatenate([v] * 8, axis=0)

    def spin_jobs(part):
        def spin(a, gate):
            l = lane
            src = x8(32 * ((l >> 2) & 3) + 16 * ((l >> 1) & 1) + 2 * (((l >> 4) - a) & 7) + (l & 1))
            for r in range(8):
                w = pltpu.bitcast(wq_raw[pl.ds(128 * r, 128), pl.ds(D * part + 128 * a, 128)], u32)
                tmp[part, a, pl.ds(64 * r, 64), :] = jnp.take_along_axis(w, src, axis=1)
        return [P_(spin, a) for a in range(8)]

    def gather_jobs(part):
        def gather(j, gate):
            l = lane
            rest = (((l >> 4) & 3) << 2) | ((l >> 6) << 1) | (l & 1)

            def col(jj, r0):
                v = tmp[part, 0, pl.ds(r0, 64), :]
                for a in range(1, 8):
                    v = jnp.where(x8(l >> 4) == ((jj + a) & 7), tmp[part, a, pl.ds(r0, 64), :], v)
                return jnp.take_along_axis(v, x8(((((l >> 1) + jj) & 7) << 4) | rest), axis=1)
            for r in range(4):
                b11, b21 = col(j, 64 * r), col(j, 256 + 64 * r)
                b12, b22 = col(j + 4, 64 * r), col(j + 4, 256 + 64 * r)
                for n, w in enumerate(_strassen_rhs(b11, b12, b21, b22)):
                    Wq[n, pl.ds(64 * r, 64), _cols(4 * part + j)] = w
        return [P_(gather, j) for j in range(4)]

    def wo_jobs():
        def stage(n, gate):
            w = pltpu.bitcast(wo_raw[:, _cols(n)], u32)
            for a in range(8):
                tmp[0, n, pl.ds(65 * a, 64), :] = w[64 * a:64 * a + 64]

        def gather(n, gate):
            for j in range(4):
                for g1 in range(2):
                    for b in range(4):
                        quad = [tmp[0, n + 4 * c, pl.ds(16 * b + 8 * g1 + j + 4 * r, 8, stride=65), :]
                                for r in range(2) for c in range(2)]
                        for q, w in enumerate(_strassen_rhs(*quad)):
                            Wo[q, pl.ds(64 * j + 32 * g1 + 8 * b, 8), _cols(n)] = w
        return [P_(stage, n) for n in range(8)] + [P_(gather, n) for n in range(4)]

    def ln_radix8(tb, g, xs):
        w = _w(jnp.concatenate(_radix8_fwd(_layernorm(xs)), axis=1))
        tb[pl.ds(8 * g, 8), :] = w
        return w

    def dft_d(r0, tb, c, gate):
        lo = _iota((T, 128), 1) < 64
        if c == 0:
            a = _dot(_b(tb[:, 0:128]), _b(gate(dm[0])))
            b = _dot(_b(tb[:, 128:256]), _b(dm[1]))
            w = _pack(jnp.where(lo, a, b), pltpu.roll(jnp.where(lo, b, a), 64, 1))
        else:
            ys, yr, yi = (_dot(_b(tb[:, _cols(n)]), _b(dm[n])) for n in range(3 * c - 1, 3 * c + 2))
            w = _pack(ys + yi if c == 1 else ys - yi, (ys - yr) * jnp.where(lo, 1.0, -1.0))
        for g in range(T // 8):
            Vp[c, pl.ds((g % 2) * 8 * PITCH + r0 // 16 + g // 2, 8, stride=PITCH), :] = w[8 * g:8 * g + 8, :]
        return w[0:8]

    def spectral(first, *R):
        def mm1(c, a, gate):
            v = Vp[c, pl.ds(a * PITCH, 128), :]
            if c == 0:
                R[c][a, 0:256, :] = _dot(_b(G[a]), _b(v))
            else:
                for h in range(2):
                    R[c][a, pl.ds(256 * h, 256), :] = _dot(_b(G[a, :, _cols(h)]), _b(v[64 * h:64 * h + 64]))

        def mid(c, g, gate):
            def load(a, r):
                v = R[c][a, pl.ds(r, 8), :]
                return v + R[c][a, pl.ds(256 + r, 8), :] if c else v
            y = _dft16([(load(a, 8 * g), load(a, 128 + 8 * g)) for a in range(16)], -1)
            if c == 0:
                part = []
                for a in range(16):
                    if g:
                        part.append(tuple(jnp.take_along_axis(load(a, o + 121 - 8 * g), 7 - sub, axis=0)
                                          for o in (0, 128)))
                    else:
                        w0 = _tw16((load(a, 0), load(a, 128)), a, -1)
                        part.append(tuple(
                            jnp.take_along_axis(jnp.where(sub == 0, p, load(a, o + 120)), (8 - sub) & 7, axis=0)
                            for p, o in zip(w0, (0, 128))))
                yneg = _dft16(part, -1)
            z = []
            for k1 in range(16):
                yr, yi = y[k1]
                w = Wf[c, pl.ds(128 * k1 + 8 * g, 8), :]
                ar, ai = _unpack(w, 0), _unpack(w, 1)
                zr, zi = yr * ar - yi * ai, yr * ai + yi * ar
                if c == 0:
                    w = Wf[4, pl.ds(128 * k1 + 8 * g, 8), :]
                    br, bi = _unpack(w, 0), _unpack(w, 1)
                    pr, pi = yneg[15 - k1]
                    zr, zi = zr + (pr * br + pi * bi), zi + (pr * bi - pi * br)
                z.append((zr, zi))
            for a, v in enumerate(_dft16(z, 1)):
                w = pltpu.bitcast(_pack(*v), f32)
                R[c][a, pl.ds(zero8 + 512 + 8 * g, 8), :] = w
            if g == 15 and c < 3 and not first:
                R[c + 1][0, pl.ds(zero8 + 640, 8), :] = w

        def mm2(c, a, gate):
            v = pltpu.bitcast(R[c][a, 512:640, :], u32)
            for h in range(2):
                u = _dot(_b(Gi[a, :, _cols(h)]), _b(v[64 * h:64 * h + 64]))
                U[2 * h, c, pl.ds(a * PITCH, 128), :] = u[:128]
                U[2 * h + 1, c, pl.ds(a * PITCH, 128), :] = u[128:]

        m1 = lambda c: [P_(mm1, c, a) for a in range(16)]
        m2 = lambda c: [P_(mm2, c, a) for a in range(16)]
        mids = lambda c: [P_(mid, c, g) for g in range(16)]

        def run(mm, vec, before=None):
            def fn():
                if before:
                    before()
                weave(mm, _spread(vec() if callable(vec) else vec, 0, len(mm)))
            region(fn)

        if first:
            def wait(*cps):
                return lambda: [cp.wait() for cp in cps]

            def merge(p, q):
                order = sorted([(n / len(p), 0, n) for n in range(len(p))]
                               + [((n + 0.5) / len(q), 1, n) for n in range(len(q))])
                return [(p, q)[src][n] for _, src, n in order]
            filt = lambda c: [P_(filter_tile, t, c) for t in range(16)]
            run(m1(0) + m1(1), lambda: gen_g(True))
            run(m1(2), filt(1), lambda: (wait(*cp_w)(), cp_q[0].start(), cp_q[1].start()))
            run(m1(3), merge(mids(1), filt(2) + filt(0)[:4]))
            run(m2(1), merge(mids(2), filt(3) + filt(0)[4:8]), lambda: (cp_q[2].start(), cp_o.start()))
            run(m2(2), merge(mids(3), filt(0)[8:]))
            run(m2(3), merge(mids(0), spin_jobs(0)), wait(cp_q[0]))
            run(m2(0), merge(gather_jobs(0), spin_jobs(1)), wait(cp_q[1]))
        else:
            run(m1(0), [])
            v = mids(0) + mids(1) + mids(2) + mids(3)
            run(m1(1) + m1(2), v[:16])
            run(m1(3) + m2(0), v[16:40])
            run(m2(1), v[40:52])
            run(m2(2), v[52:])
            run(m2(3), [])

    def run_spectral(first):
        pl.run_scoped(P_(spectral, first), *[pltpu.VMEM((16, 648, 128), f32)] * 4)

    def rowwise(last, ub, ya, yb, zf, o0, o1, z0, z1, QK0, QK1, VO0, VO1):
        bufs = ((QK0, VO0), (QK1, VO1))

        def idft_operands(r0, c, gate):
            def get(q):
                return jnp.concatenate(
                    [U[q, c, pl.ds(r0 // 16 + g, 16, stride=PITCH), :]
                     + U[q + 2, c, pl.ds(r0 // 16 + g, 16, stride=PITCH), :] for g in range(T // 16)], axis=0)
            lo = _iota((T, 128), 1) < 64
            ur, ui = gate(get(0)), get(1)
            if c == 0:
                ui = pltpu.roll(ui, 64, 1)
                ops = jnp.where(lo, ur, ui), jnp.where(lo, ui, ur)
            else:
                ui = ui * jnp.where(lo, 1.0, -1.0)
                ops = ur + ui, ui, ur
            for n, u in enumerate(ops):
                w = _w(u)
                ub[:, _cols(max(3 * c - 1, 0) + n)] = w
            return w[-8:]

        def idft_d(ya, c, gate):
            if c == 0:
                ya[:, 0:128] = _dot_nt(_b(ub[:, 0:128]), _b(gate(dm[0])))
                y = _dot_nt(_b(ub[:, 128:256]), _b(dm[1]))
            else:
                ys, yi, yr = (_dot_nt(_b(ub[:, _cols(n)]), _b(dm[n])) for n in range(3 * c - 1, 3 * c + 2))
                ya[:, _cols(2 * c)] = ys - yi
                y = yr - ys if c == 1 else ys - yr
            ya[:, _cols(2 * c + 1)] = y
            return y[0:8]

        def ln_attn(r0, ya, g, gate):
            rr, rows = pl.ds(r0 + 16 * g, 16), pl.ds(16 * g, 16)
            yt = _tiles(ya[rows, :])
            yt[0] = gate(yt[0])
            x0 = X2[rr, :] if last else xin[rr, :].astype(f32)
            xs = [a + b for a, b in zip(_tiles(x0), _radix8_inv(yt))]
            X[rr, :] = jnp.concatenate(xs, axis=1)
            z = jnp.concatenate(_layernorm(xs), axis=1)
            zf[rows, :] = z
            return z

        def operands(get, dst, g, gate):
            top, bot = get(pl.ds(16 * g, 16)), get(pl.ds(H + 16 * g, 16))
            top[0] = gate(top[0])
            for q, a in enumerate(_strassen_lhs(top, bot)):
                w = _w(a)
                dst[q, pl.ds(8 * g, 8), :] = w
            return w

        def strassen(A, B, n, put):
            m = {}

            def mm(q, gate=lambda v: v):
                return _dot(_b(A[q]), _b(gate(B[q, :, _cols(n)])))

            def first(gate):
                m[1], m[2], m[3] = mm(0, gate), mm(1), mm(2)
                c22 = ((m[1] - m[2]) + m[3]) + mm(5)
                put(1, 1, c22)
                return c22[0:8]

            def second(gate):
                m4 = mm(3, gate)
                put(1, 0, m[2] + m4)
                m5 = mm(4)
                put(0, 1, m[3] + m5)
                c11 = ((m[1] + m4) - m5) + mm(6)
                put(0, 0, c11)
                return c11[0:8]
            return [first, second]

        def proj(z, par, n):
            part = n // 4
            dst, t0 = bufs[par][part >> 1], 8 * (part & 1)

            def put(r, c, y):
                dst[t0 + 4 * c + n % 4, pl.ds(16 + r * H, H), :] = y
            return strassen(z, Wq, n, put)

        def softmax(r0, par, rr, gate):
            QK = bufs[par][0]
            q = [QK[j, pl.ds(16 + rr, 8), :] for j in range(8)]
            q[0] = gate(q[0])
            L = []
            for w in range(8):
                p = _tree(jnp.add, [q[j] * QK[8 + j, pl.ds(16 + rr - 2 * w, 8), :] for j in range(8)])
                p = p + pltpu.roll(p, 64, 1)
                p = p + jnp.take_along_axis(p, lane ^ 1, axis=1)
                if rr < 2 * w:
                    p = jnp.where(r0 + rr + sub >= 2 * w, p, -1e9 * 32 ** 0.5)
                L.append(p)
            m = _tree(jnp.maximum, L)
            e = [jnp.exp2((l - m) * float(32 ** -0.5 * np.log2(np.e))) for l in L]
            inv = 1.0 / _tree(jnp.add, e)
            return [v * inv for v in e]

        def mix(par, rr, z8, p):
            VO = bufs[par][1]
            for j in range(8):
                o = _tree(jnp.add, [p[w] * VO[j, pl.ds(16 + rr - 2 * w, 8), :] for w in range(8)])
                VO[8 + j, pl.ds(z8 + rr, 8), :] = o
            return o

        def attend(r0, par, rr, ordered, gate):
            p = softmax(r0, par, rr, gate)
            if ordered:
                QK = bufs[par][0]
                for w in range(8):
                    QK[16 + w, pl.ds(zero8 + rr, 8), :] = p[w]
                p = [QK[16 + w, pl.ds(rr, 8), :] for w in range(8)]
            return mix(par, rr, zero8 if ordered else 0, p)

        def out_proj(r0, ob, yb, n):
            def put(r, c, y):
                at = (pl.ds(r0 + r * H, H), _cols(4 * c + n))
                if last:
                    xin[at] = (X[at] + y).astype(bf16)
                else:
                    yb[pl.ds(r * H, H), _cols(4 * c + n)] = X[at] + y
            return strassen(ob, Wo, n, put)

        def residual(r0, tb, yb, g, gate):
            v = gate(yb[pl.ds(16 * g, 16), :])
            X2[pl.ds(r0 + 16 * g, 16), :] = v
            return ln_radix8(tb, g, _tiles(v))

        def in_pairs(fn):
            def job(cs, gate):
                return [fn(c, gate if c == cs[0] else (lambda v: v)) for c in cs][-1]
            return [P_(job, (0, 1)), P_(job, (2, 3))]
        m_idft = lambda y=ya: in_pairs(P_(idft_d, y))
        v_iop = lambda r0: [P_(idft_operands, r0, c) for c in range(4)]
        m_proj = lambda par, lo=0, hi=12: [j for n in range(lo, hi) for j in proj((z0, z1)[par], par, n)]
        m_out = lambda r0, ob, y=yb: [j for n in range(4) for j in out_proj(r0, ob, y, n)]
        m_dft = lambda r0, tb=tb0: [] if last else in_pairs(P_(dft_d, r0, tb))

        def v_ln(r0, par, y=ya):
            jobs = []
            for g in range(H // 16):
                jobs += [P_(ln_attn, r0, y, g), P_(ln_attn, r0, y, g + H // 16),
                         P_(operands, lambda rows: _tiles(zf[rows, :]), (z0, z1)[par], g)]
            return jobs

        def v_att(r0, par, ordered=True, dst=None):
            jobs = []
            for g in range(H // 16):
                jobs += [P_(attend, r0, par, h + 16 * g + e, ordered) for h in (0, H) for e in (0, 8)]
                jobs += [P_(operands, lambda rows: [bufs[par][1][8 + j, rows, :] for j in range(8)],
                            (o0, o1)[par] if dst is None else dst, g)]
            return jobs
        v_res = lambda r0, tb=tb0, y=yb: [] if last else [P_(residual, r0, tb, y, g) for g in range(T // 16)]

        def halo(par, first=False):
            for j in range(8):
                for dst, src, t in zip(bufs[par], bufs[1 - par], (8 + j, j)):
                    dst[t, 0:16, :] = jnp.zeros((16, 128), f32) if first else src[t, T:T + 16, :]

        def head0():
            halo(0, True)
            weave(m_idft(yb) + m_idft(),
                  _spread(v_iop(0), 0, 0) + _spread(v_iop(T), 2, 2) + _spread(v_ln(0, 0, yb), 2, 4))

        def head(part):
            if part < 2:
                (cp_q[2], cp_o)[part].wait()
            vec = (_spread(gather_jobs(1), 0, 8) + _spread(spin_jobs(2), 0, 8),
                   _spread(gather_jobs(2), 0, 8) + _spread(wo_jobs()[:8], 0, 8),
                   _spread(wo_jobs()[8:], 0, 8))[part]
            weave(m_proj(0, 4 * part, 4 * part + 4), vec + _spread(v_ln(T, 1)[8 * part:8 * part + 8], 0, 8))

        def step(i, par, old=True):
            rn, rp, ro = ((i + d) * T if isinstance(i, int) else pl.multiple_of((i + d) * T, T) for d in (1, -1, -2))
            halo(par)
            mo, mi = m_out(ro, (o0, o1)[par]) if old else [], m_idft()
            a, b = len(mo), len(mo) + len(mi)
            na, nl = (26, 24) if old and not last else (22, 22)
            vec = _spread(v_att(rp, 1 - par), 0, b + na, 4 if old else 3)
            if old:
                vec += _spread(v_res(ro), a, b + 22, 2)
            vec += _spread(v_iop(rn), 0, a, 2 if old else None)
            vec += _spread(v_ln(rn, 1 - par), b, b + nl, 2)
            p, md = m_proj(par), m_dft(ro) if old else []
            weave(mo + mi + p[:22] + md + p[22:], vec)
            if last and old:
                out_copy(ro, i - 2).start()

        r5, r6, r7 = ((NB - d) * T for d in (3, 2, 1))

        def tail0():
            halo(1)
            weave(m_proj(1), _spread(v_att(r6, 0), 0, 22, 4))

        def tail1():
            weave(m_out(r5, o1, ya) + m_out(r6, o0) + m_dft(r5),
                  _spread(v_att(r7, 1, False, z0), 0, 14, 4) + _spread(v_res(r5, tb0, ya), 8, 16, 2))
            if last:
                out_copy(r5, NB - 3).start()
                out_copy(r6, NB - 2).start()

        def tail2():
            weave(m_out(r7, z0, ya) + m_dft(r6), _spread(v_res(r6), 0, 7, 2))
            if last:
                out_copy(r7, NB - 1).start()
            for job in v_res(r7, tb1, ya):
                job(lambda v: v)
            weave(m_dft(r7, tb1), [])

        def head_all():
            weave(m_proj(0), _spread(v_ln(T, 1), 0, 22, 2))
        heads = [head_all] if last else [P_(head, part) for part in range(3)]
        for fn in [head0] + heads + [P_(step, 1, 1, False)]:
            region(fn)

        def loop(i, _):
            for par in range(2):
                pl.when(i % 2 == par)(P_(step, i, par))
            return _
        jax.lax.fori_loop(2, NB - 1, loop, 0)
        for fn in (tail0, tail1, tail2):
            region(fn)

    def run_rowwise(last):
        zs = pltpu.VMEM((7, H // 2, 512), u32)
        rows, qk, vo = pltpu.VMEM((T, D), f32), pltpu.VMEM((24, 16 + T, 128), f32), pltpu.VMEM((16, 16 + T, 128), f32)
        pl.run_scoped(P_(rowwise, last), pltpu.VMEM((T // 2, 11 * 128), u32),
                      rows, rows, rows, zs, zs, zs, zs, qk, qk, vo, vo)

    gen_dm()

    def ln_x(r0, tb, g, gate):
        return ln_radix8(tb, g, _tiles(xin[pl.ds(r0 + 16 * g, 16), :].astype(f32)))

    def first_dft(i, par):
        r0 = pl.multiple_of(i * T, T)
        x_copy(r0, i).wait()

        @pl.when(i + 3 < NB)
        def _():
            x_copy(pl.multiple_of(jnp.minimum(i + 3, NB - 1) * T, T), jnp.minimum(i + 3, NB - 1)).start()

        @pl.when(i + 3 == NB)
        def _():
            for cp in cp_w:
                cp.start()
        weave([P_(dft_d, r0 - T, (tb0, tb1)[1 - par], c) for c in range(4)],
              _spread([P_(ln_x, r0, (tb0, tb1)[par], g) for g in range(T // 16)], 0, 4, 2))

    def first_ln():
        x_copy(0, 0).wait()
        x_copy(3 * T, 3).start()
        weave([], _spread([P_(ln_x, 0, tb0, g) for g in range(T // 16)], 0, 0))

    def first_loop(i, _):
        for par in range(2):
            pl.when(i % 2 == par)(P_(first_dft, i, par))
        return _

    region(first_ln)
    jax.lax.fori_loop(1, NB, first_loop, 0)
    region(lambda: weave([P_(dft_d, (NB - 1) * T, tb1, c) for c in range(4)], _spread(gen_g(False), 0, 4)))
    run_spectral(True)
    run_rowwise(False)
    run_spectral(False)
    run_rowwise(True)
    for i in range(NB):
        out_copy(i * T, i).wait()


@jax.jit
def pallas_interleave_layers__spectral_gfnet__sliding_local_dilated__prompt_kernel(
        A_x, A_w_r, A_w_i, B_x, B_wqkv, B_wo):
    del B_x
    hbm = pl.BlockSpec(memory_space=pltpu.HBM)
    args = (A_x.reshape(S, D), A_w_r.T, A_w_i.T, B_wqkv, B_wo, jnp.asarray(_seeds()))
    out = pl.pallas_call(
        _kernel,
        out_shape=jax.ShapeDtypeStruct((S, D), bf16),
        in_specs=[hbm] * 6,
        out_specs=hbm,
        scratch_shapes=[
            pltpu.VMEM((34, 8, 128), f32),
            pltpu.VMEM((S, D), bf16),
            pltpu.VMEM((S, D), f32),
            pltpu.VMEM((S, D), f32),
            pltpu.VMEM((4, 17 * PITCH - 1, 128), u32),
            pltpu.VMEM((4, 4, 17 * PITCH - 1, 128), f32),
            pltpu.VMEM((11, 64, 128), u32),
            pltpu.VMEM((16, 128, 256), u32),
            pltpu.VMEM((16, 128, 256), u32),
            pltpu.VMEM((5, S, 128), u32),
            pltpu.VMEM((7, 256, 1536), u32),
            pltpu.VMEM((7, 256, 512), u32),
            pltpu.VMEM((T // 2, 11 * 128), u32),
            pltpu.VMEM((T // 2, 11 * 128), u32),
            pltpu.VMEM((513, S), bf16),
            pltpu.VMEM((513, S), bf16),
            pltpu.VMEM((D, 3 * D), bf16),
            pltpu.VMEM((D, D), bf16),
            pltpu.VMEM((3, 8, 584, 128), u32),
            pltpu.VMEM((16, 520, 128), u32),
            pltpu.SemaphoreType.DMA((NB + 9,)),
        ],
        compiler_params=pltpu.CompilerParams(vmem_limit_bytes=127 * 1024 * 1024),
    )(*args)
    return out.reshape(1, S, D)
```

```python
import functools
import numpy as np
import jax
import jax.numpy as jnp
from jax.experimental import pallas as pl
from jax.experimental.pallas import tpu as pltpu

S, D = 2048, 1024
f32, bf16, u32 = jnp.float32, jnp.bfloat16, jnp.uint32
T = 256
NB = S // T
H = T // 2
VPITCH = 65
PITCH = 129
R2 = float(np.sqrt(0.5))
SCALE = 2.0 / (S * D)


def _seeds():
    r = np.arange(8)[:, None]
    l = np.arange(128)[None, :]
    cls, j = l >> 6, l & 63
    tiles = []
    freqs = [8 * j, 8 * j + 4] + [8 * j + np.where(cls == 0, c, 8 - c) for c in (1, 2, 3)]
    for m in freqs:
        th, st = 2 * np.pi * r * m / D, 2 * np.pi * 8 * m / D + 0 * r
        tiles += [np.cos(th), np.sin(th), np.cos(st), np.sin(st)]
    for h in range(2):
        col = 128 * h + l
        b, odd = col >> 1, (col & 1) == 1
        al, st, tw = 2 * np.pi * r * b / 128, 2 * np.pi * 8 * b / 128 + 0 * r, 2 * np.pi * b / S + 0 * r
        tiles += [np.where(odd, np.sin(al), np.cos(al)), np.where(odd, np.cos(al), -np.sin(al)),
                  np.cos(st), np.sin(st), np.cos(tw), np.sin(tw)]
    tw = 2 * np.pi * r / S + 0 * l
    al, st = 2 * np.pi * r * l / 128, 2 * np.pi * 8 * l / 128 + 0 * r
    tiles += [np.cos(tw), np.sin(tw), np.cos(al), np.sin(al), np.cos(st), np.sin(st)]
    return np.stack(tiles).astype(np.float32)


def _iota(shape, axis):
    return jax.lax.broadcasted_iota(jnp.int32, shape, axis)


def _pack(a, b):
    return pltpu.pack_elementwise([a, b], packed_dtype=bf16)


def _unpack(w, i):
    return pltpu.unpack_elementwise(w, index=i, packed_dtype=bf16, unpacked_dtype=f32)


def _tiles(v):
    return [v[:, 128 * a:128 * (a + 1)] for a in range(v.shape[1] // 128)]


def _tree(op, xs):
    xs = list(xs)
    while len(xs) > 1:
        xs = [op(xs[i], xs[i + 1]) if i + 1 < len(xs) else xs[i] for i in range(0, len(xs), 2)]
    return xs[0]


def _rot(c, s, cs, ss):
    return c * cs - s * ss, s * cs + c * ss


def _layernorm(xs):
    m = jnp.sum(_tree(jnp.add, xs), axis=-1, keepdims=True) * (1.0 / D)
    xc = [x - m for x in xs]
    v = jnp.sum(_tree(jnp.add, [x * x for x in xc]), axis=-1, keepdims=True) * (1.0 / D)
    inv = jax.lax.rsqrt(v + 1e-5)
    return [x * inv for x in xc]


def _radix8_fwd(z):
    e = [z[a] + z[a + 4] for a in range(4)]
    o = [z[a] - z[a + 4] for a in range(4)]
    s02, s13 = e[0] + e[2], e[1] + e[3]
    p, q = (o[1] - o[3]) * R2, (o[1] + o[3]) * R2
    r1, n1, r2, i2, r3, i3 = o[0] + p, o[2] + q, e[0] - e[2], e[3] - e[1], o[0] - p, o[2] - q
    return [s02 + s13, s02 - s13, r1 - n1, r1, n1, r2 + i2, r2, i2, r3 + i3, r3, i3]


def _radix8_inv(t):
    t0, t4, r1, n1, r2, i2, r3, i3 = t
    a, b = t0 + t4, t0 - t4
    E = [a + r2, b - i2, a - r2, b + i2]
    u, v = r1 - r3, i3 - n1
    O = [r1 + r3, (u - v) * R2, i3 + n1, (u + v) * (-R2)]
    return [E[k] + O[k] for k in range(4)] + [E[k] - O[k] for k in range(4)]


def _dft4(x, sgn):
    (ar, ai), (br, bi), (cr, ci), (dr, di) = x
    sr, si, tr, ti = ar + cr, ai + ci, ar - cr, ai - ci
    ur, ui, vr, vi = br + dr, bi + di, br - dr, bi - di
    y1, y3 = (tr + vi, ti - vr), (tr - vi, ti + vr)
    if sgn > 0:
        y1, y3 = y3, y1
    return [(sr + ur, si + ui), y1, (sr - ur, si - ui), y3]


def _tw16(x, k, sgn):
    xr, xi = x
    k = k % 16
    if k == 0:
        return x
    if k == 4:
        return (xi, -xr) if sgn < 0 else (-xi, xr)
    if k == 2:
        return ((xr + xi) * R2, (xi - xr) * R2) if sgn < 0 else ((xr - xi) * R2, (xi + xr) * R2)
    if k == 6:
        return ((xi - xr) * R2, (xr + xi) * (-R2)) if sgn < 0 else ((xr + xi) * (-R2), (xr - xi) * R2)
    c, s = float(np.cos(np.pi * k / 8)), float(sgn * np.sin(np.pi * k / 8))
    return (xr * c - xi * s, xi * c + xr * s)


def _dft16(x, sgn):
    cols = [_dft4([x[a2 + 4 * a1] for a1 in range(4)], sgn) for a2 in range(4)]
    out = [None] * 16
    for k1 in range(4):
        y = _dft4([_tw16(cols[a2][k1], a2 * k1, sgn) for a2 in range(4)], sgn)
        for k2 in range(4):
            out[k1 + 4 * k2] = y[k2]
    return out


def _dot(a, b):
    return jnp.dot(a, b, preferred_element_type=f32)


def _dot_nt(a, b):
    return jax.lax.dot_general(a, b, (((1,), (1,)), ((), ())), preferred_element_type=f32)


def _b(w):
    return pltpu.bitcast(w, bf16)


def _w(v):
    return pltpu.bitcast(v.astype(bf16), u32)


def _strassen_lhs(top, bot):
    a11, a12 = jnp.concatenate(top[:4], axis=1), jnp.concatenate(top[4:], axis=1)
    a21, a22 = jnp.concatenate(bot[:4], axis=1), jnp.concatenate(bot[4:], axis=1)
    return [a11 + a22, a21 + a22, a11, a22, a11 + a12, a21 - a11, a12 - a22]


def _strassen_rhs(b11, b12, b21, b22):
    def comb(p, q, op):
        return _pack(op(_unpack(p, 0), _unpack(q, 0)), op(_unpack(p, 1), _unpack(q, 1)))
    return [comb(b11, b22, jnp.add), b11, comb(b12, b22, jnp.subtract), comb(b21, b11, jnp.subtract),
            b22, comb(b11, b12, jnp.add), comb(b21, b22, jnp.add)]


def _weave(never, mm, vec):
    def gate(tokens):
        def apply(v):
            if not tokens:
                return v
            t = v[0:8, 0:128]
            tok = _tree(jnp.bitwise_or, [k if k.dtype == u32 else pltpu.bitcast(k, u32) for k in tokens])
            t = jnp.where(never, tok if t.dtype == u32 else pltpu.bitcast(tok, t.dtype), t)
            if v.shape[1] > 128:
                t = jnp.concatenate([t, v[0:8, 128:]], axis=1)
            return jnp.concatenate([t, v[8:]], axis=0) if v.shape[0] > 8 else t
        return apply
    done, due = {}, {}
    for n in range(-1, len(mm)):
        if n >= 0:
            done[n] = mm[n](gate(due.pop(n, [])))
        for job, after, before in vec:
            if max(after, -1) == n:
                tied = before is not None
                tok = job(gate([done[n]] if tied and n >= 0 else []))
                if tied:
                    due.setdefault(before, []).append(tok[0:8, 0:128])


def _spread(jobs, lo, hi, window=None):
    out = []
    for k, job in enumerate(jobs):
        n = lo + (k * (hi - lo)) // len(jobs)
        out.append((job, n - 1, None if window is None else min(n + window, hi)))
    return out


def _cols(j, n=1):
    return pl.ds(128 * j, 128 * n)


def _kernel(x_hbm, wr_hbm, wi_hbm, wqkv_hbm, wo_hbm, seed_hbm, out_hbm,
            seed, xin, X, X2, Vp, U, dm, G, Gi, Wf, Wq, Wo, tb0, tb1, wr, wi, wq_raw, wo_raw, tmp, WE, sem):
    P_ = functools.partial
    sub = _iota((8, 128), 0)
    lane = _iota((8, 128), 1)
    lane16 = _iota((16, 128), 1)

    def x_copy(r0, i):
        return pltpu.make_async_copy(x_hbm.at[pl.ds(r0, T)], xin.at[pl.ds(r0, T)], sem.at[i])

    def out_copy(r0, i):
        return pltpu.make_async_copy(xin.at[pl.ds(r0, T)], out_hbm.at[pl.ds(r0, T)], sem.at[i])

    cp_seed = pltpu.make_async_copy(seed_hbm, seed, sem.at[NB])
    cp_w = [pltpu.make_async_copy(src, dst, sem.at[NB + 1 + q])
            for q, (src, dst) in enumerate(((wr_hbm, wr), (wi_hbm, wi)))]
    cp_q = [pltpu.make_async_copy(wqkv_hbm.at[:, pl.ds(D * n, D)], wq_raw.at[:, pl.ds(D * n, D)],
                                  sem.at[NB + 5 + n]) for n in range(3)]
    cp_o = pltpu.make_async_copy(wo_hbm, wo_raw, sem.at[NB + 8])
    cp_seed.start()
    x_copy(0, 0).start()
    x_copy(T, 1).start()
    cp_seed.wait()
    x_copy(2 * T, 2).start()

    zero = (seed[0] > 2.0).astype(jnp.int32)[0, 0]
    zero8 = pl.multiple_of(8 * zero, 8)
    regions = []

    def region(fn):
        regions.append(fn)
        pl.when(zero < len(regions))(fn)

    def weave(mm, vec):
        _weave(seed[0] > 2.0, mm, vec)

    def gen_dm():
        lo = lane16 < 64
        for n in range(5):
            c, s, cs, ss = (seed[4 * n + q] for q in range(4))
            for g in range(8):
                c2, s2 = _rot(c, s, cs, ss)
                cc, sc = jnp.concatenate([c, c2], axis=0), jnp.concatenate([s, s2], axis=0)
                rows = pl.ds(8 * g, 8)
                if n == 0:
                    alt = (1 - 2 * (_iota((16, 128), 0) & 1)).astype(f32)
                    dm[0, rows, :] = _w(jnp.where(lane16 == 64, alt, jnp.where(lo, cc, -sc)))
                elif n == 1:
                    dm[1, rows, :] = _w(jnp.where(lo, -sc, cc))
                else:
                    sc = jnp.where(lo, sc, -sc)
                    dm[3 * n - 4, rows, :] = _w(cc)
                    dm[3 * n - 3, rows, :] = _w(cc + sc)
                    dm[3 * n - 2, rows, :] = _w(cc - sc)
                if g < 7:
                    c, s = _rot(c2, s2, cs, ss)

    def gen_g(inverse):
        st = dict(pq=[seed[20], seed[21], seed[26], seed[27]], cs=(seed[34], seed[35]), tw=(seed[32], seed[33]))
        c1, s1 = float(np.cos(2 * np.pi * 8 / S)), float(np.sin(2 * np.pi * 8 / S))
        rows2 = lambda p, q: tuple(jnp.concatenate(v, axis=0) for v in zip(p, q))

        def forward(g, gate):
            tw1, cs1 = _rot(*st['tw'], c1, s1), _rot(*st['cs'], seed[36], seed[37])
            (cb, sb), (c, s) = rows2(st['tw'], tw1), rows2(st['cs'], cs1)
            st['tw'], st['cs'] = _rot(*tw1, c1, s1), _rot(*cs1, seed[36], seed[37])
            for a in range(16):
                for n, v in enumerate((c, c + s, c - s)):
                    G[a, n, pl.ds(8 * g, 8), :] = _w(v)
                if a < 15:
                    c, s = _rot(c, s, cb, sb)

        def backward(g, gate):
            for h in range(2):
                p0, q0 = st['pq'][2 * h:2 * h + 2]
                cs, ss, ct, sn = (seed[22 + 6 * h + n] for n in range(4))
                q1, p1 = _rot(q0, p0, cs, ss)
                p, q = rows2((p0, q0), (p1, q1))
                st['pq'][2 * h + 1], st['pq'][2 * h] = _rot(q1, p1, cs, ss)
                sg = (1 - 2 * (lane16 & 1)).astype(f32) * SCALE
                p, q = p * sg, q * (-sg)
                ct, sn = rows2((ct, sn), (ct, sn))
                for a in range(16):
                    Gi[a, pl.ds(8 * g, 8), _cols(h)] = _w(p)
                    Gi[a, pl.ds(64 + 8 * g, 8), _cols(h)] = _w(q)
                    if a < 15:
                        p, q = _rot(p, q, ct, sn)
        return [P_(backward if inverse else forward, g) for g in range(8)]

    def filter_tile(t, c, gate):
        we = WE.at[t]
        if c == 1:
            a = pltpu.bitcast(wr[0:512, _cols(t)], u32)
            b = pltpu.bitcast(wi[0:512, _cols(t)], u32)
            we[0:256] = (a & 0xFFFF) | (b << 16)
            we[256:512] = (a >> 16) | (b & jnp.uint32(0xFFFF0000))
        w = jnp.concatenate([we[pl.ds(256 * (r & 1) + (r >> 1), 64, stride=4), :]
                             for r in (c, (8 - c) if c else 4)], axis=0)
        if c == 0:
            def rows(src_t):
                return [jnp.broadcast_to(src[m:m + 1, _cols(src_t)].astype(f32), (8, 128))
                        for m in (0, D // 2) for src in (wr, wi)]
            ar, ai, br, bi = rows(t)
            cr, ci, dr, di = (jnp.take_along_axis(jnp.where(lane == 0, p, q), (128 - lane) & 127, axis=1)
                              for p, q in zip(rows((16 - t) % 16), rows(15 - t)))
            same = _pack(((ar + br) + (cr + dr)) * 0.125, ((ai + bi) - (ci + di)) * 0.125)
            pair = _pack(((ar - br) + (cr - dr)) * 0.125, ((ai - bi) - (ci - di)) * 0.125)
            w = jnp.concatenate([jnp.where(sub == 0, same, w[0:8]), w[8:]], axis=0)
            p = jnp.concatenate([jnp.where(sub == 0, pair, 0), jnp.zeros((120, 128), u32)], axis=0)
            Wf[4, pl.ds(128 * t, 128), :] = p.T
        Wf[c, pl.ds(128 * t, 128), :] = w.T

    x8 = lambda v: jnp.concatenate([v] * 8, axis=0)

    def spin_jobs(part):
        def spin(a, gate):
            l = lane
            src = x8(32 * ((l >> 2) & 3) + 16 * ((l >> 1) & 1) + 2 * (((l >> 4) - a) & 7) + (l & 1))
            for r in range(8):
                w = pltpu.bitcast(wq_raw[pl.ds(128 * r, 128), pl.ds(D * part + 128 * a, 128)], u32)
                tmp[part, a, pl.ds(64 * r, 64), :] = jnp.take_along_axis(w, src, axis=1)
        return [P_(spin, a) for a in range(8)]

    def gather_jobs(part):
        def gather(j, gate):
            l = lane
            rest = (((l >> 4) & 3) << 2) | ((l >> 6) << 1) | (l & 1)

            def col(jj, r0):
                v = tmp[part, 0, pl.ds(r0, 64), :]
                for a in range(1, 8):
                    v = jnp.where(x8(l >> 4) == ((jj + a) & 7), tmp[part, a, pl.ds(r0, 64), :], v)
                return jnp.take_along_axis(v, x8(((((l >> 1) + jj) & 7) << 4) | rest), axis=1)
            for r in range(4):
                b11, b21 = col(j, 64 * r), col(j, 256 + 64 * r)
                b12, b22 = col(j + 4, 64 * r), col(j + 4, 256 + 64 * r)
                for n, w in enumerate(_strassen_rhs(b11, b12, b21, b22)):
                    Wq[n, pl.ds(64 * r, 64), _cols(4 * part + j)] = w
        return [P_(gather, j) for j in range(4)]

    def wo_jobs():
        def stage(n, gate):
            w = pltpu.bitcast(wo_raw[:, _cols(n)], u32)
            for a in range(8):
                tmp[0, n, pl.ds(65 * a, 64), :] = w[64 * a:64 * a + 64]

        def gather(n, gate):
            for j in range(4):
                for g1 in range(2):
                    for b in range(4):
                        quad = [tmp[0, n + 4 * c, pl.ds(16 * b + 8 * g1 + j + 4 * r, 8, stride=65), :]
                                for r in range(2) for c in range(2)]
                        for q, w in enumerate(_strassen_rhs(*quad)):
                            Wo[q, pl.ds(64 * j + 32 * g1 + 8 * b, 8), _cols(n)] = w
        return [P_(stage, n) for n in range(8)] + [P_(gather, n) for n in range(4)]

    def ln_radix8(tb, g, xs):
        w = _w(jnp.concatenate(_radix8_fwd(_layernorm(xs)), axis=1))
        tb[pl.ds(8 * g, 8), :] = w
        return w

    def dft_d(r0, tb, c, gate):
        lo = _iota((T, 128), 1) < 64
        if c == 0:
            a = _dot(_b(tb[:, 0:128]), _b(gate(dm[0])))
            b = _dot(_b(tb[:, 128:256]), _b(dm[1]))
            re, im = jnp.where(lo, a, b), pltpu.roll(jnp.where(lo, b, a), 64, 1)
        else:
            ys, yr, yi = (_dot(_b(tb[:, _cols(n)]), _b(dm[n])) for n in range(3 * c - 1, 3 * c + 2))
            re, im = ys + yi if c == 1 else ys - yi, (ys - yr) * jnp.where(lo, 1.0, -1.0)
        for n, v in enumerate((re + im, re, im)):
            for g in range(T // 32):
                for h in (0, 8):
                    w = _pack(v[32 * g + h:32 * g + h + 8], v[32 * g + h + 16:32 * g + h + 24])
                    Vp[c, n, pl.ds(h * VPITCH + r0 // 32 + g, 8, stride=VPITCH), :] = w
        return w

    def spectral(first, *R):
        def mm1(c, a, gate):
            for n in range(3):
                R[c][a, pl.ds(128 * n, 128), :] = _dot(_b(G[a, n]), _b(Vp[c, n, pl.ds(a * VPITCH, 64), :]))

        def mid(c, g, gate):
            def load(a, r):
                ys, yr, yi = (R[c][a, pl.ds(128 * n + r, 8), :] for n in range(3))
                return ys - yi, ys - yr
            y = _dft16([load(a, 8 * g) for a in range(16)], -1)
            if c == 0:
                part = []
                for a in range(16):
                    if g:
                        part.append(tuple(jnp.take_along_axis(v, 7 - sub, axis=0) for v in load(a, 121 - 8 * g)))
                    else:
                        part.append(tuple(
                            jnp.take_along_axis(jnp.where(sub == 0, p, q), (8 - sub) & 7, axis=0)
                            for p, q in zip(_tw16(load(a, 0), a, -1), load(a, 120))))
                yneg = _dft16(part, -1)
            z = []
            for k1 in range(16):
                yr, yi = y[k1]
                w = Wf[c, pl.ds(128 * k1 + 8 * g, 8), :]
                ar, ai = _unpack(w, 0), _unpack(w, 1)
                zr, zi = yr * ar - yi * ai, yr * ai + yi * ar
                if c == 0:
                    w = Wf[4, pl.ds(128 * k1 + 8 * g, 8), :]
                    br, bi = _unpack(w, 0), _unpack(w, 1)
                    pr, pi = yneg[15 - k1]
                    zr, zi = zr + (pr * br + pi * bi), zi + (pr * bi - pi * br)
                z.append((zr, zi))
            for a, v in enumerate(_dft16(z, 1)):
                w = pltpu.bitcast(_pack(*v), f32)
                R[c][a, pl.ds(zero8 + 512 + 8 * g, 8), :] = w
            if g == 15 and c < 3 and not first:
                R[c + 1][0, pl.ds(zero8 + 640, 8), :] = w

        def mm2(c, a, gate):
            v = pltpu.bitcast(R[c][a, 512:640, :], u32)
            for h in range(2):
                u = _dot(_b(Gi[a, :, _cols(h)]), _b(v[64 * h:64 * h + 64]))
                U[2 * h, c, pl.ds(a * PITCH, 128), :] = u[:128]
                U[2 * h + 1, c, pl.ds(a * PITCH, 128), :] = u[128:]

        m1 = lambda c: [P_(mm1, c, a) for a in range(16)]
        m2 = lambda c: [P_(mm2, c, a) for a in range(16)]
        mids = lambda c: [P_(mid, c, g) for g in range(16)]

        def run(mm, vec, before=None):
            def fn():
                if before:
                    before()
                weave(mm, _spread(vec() if callable(vec) else vec, 0, len(mm)))
            region(fn)

        if first:
            def wait(*cps):
                return lambda: [cp.wait() for cp in cps]

            def merge(p, q):
                order = sorted([(n / len(p), 0, n) for n in range(len(p))]
                               + [((n + 0.5) / len(q), 1, n) for n in range(len(q))])
                return [(p, q)[src][n] for _, src, n in order]
            filt = lambda c: [P_(filter_tile, t, c) for t in range(16)]
            run(m1(0) + m1(1), lambda: gen_g(True))
            run(m1(2), filt(1), wait(*cp_w))
            run(m1(3), merge(mids(1), filt(2) + filt(0)[:6]), cp_q[0].start)
            run(m2(1), merge(mids(2), filt(3) + filt(0)[6:12]), cp_q[1].start)
            run(m2(2), merge(mids(3), filt(0)[12:] + spin_jobs(0)[:3]),
                lambda: (cp_q[0].wait(), cp_q[2].start()))
            run(m2(3), merge(mids(0), spin_jobs(0)[3:]), cp_o.start)
            run(m2(0), merge(gather_jobs(0), spin_jobs(1)), cp_q[1].wait)
        else:
            run(m1(0), [])
            v = mids(0) + mids(1) + mids(2) + mids(3)
            run(m1(1) + m1(2), v[:16])
            run(m1(3) + m2(0), v[16:40])
            run(m2(1), v[40:52])
            run(m2(2), v[52:])
            run(m2(3), [])

    def run_spectral(first):
        pl.run_scoped(P_(spectral, first), *[pltpu.VMEM((16, 648, 128), f32)] * 4)

    def rowwise(last, ub, ya, yb, zf, o0, o1, z0, z1, QK0, QK1, VO0, VO1):
        bufs = ((QK0, VO0), (QK1, VO1))

        def idft_operands(r0, c, gate):
            def get(q):
                return jnp.concatenate(
                    [U[q, c, pl.ds(r0 // 16 + g, 16, stride=PITCH), :]
                     + U[q + 2, c, pl.ds(r0 // 16 + g, 16, stride=PITCH), :] for g in range(T // 16)], axis=0)
            lo = _iota((T, 128), 1) < 64
            ur, ui = gate(get(0)), get(1)
            if c == 0:
                ui = pltpu.roll(ui, 64, 1)
                ops = jnp.where(lo, ur, ui), jnp.where(lo, ui, ur)
            else:
                ui = ui * jnp.where(lo, 1.0, -1.0)
                ops = ur + ui, ui, ur
            for n, u in enumerate(ops):
                w = _w(u)
                ub[:, _cols(max(3 * c - 1, 0) + n)] = w
            return w[-8:]

        def idft_d(ya, c, gate):
            if c == 0:
                ya[:, 0:128] = _dot_nt(_b(ub[:, 0:128]), _b(gate(dm[0])))
                y = _dot_nt(_b(ub[:, 128:256]), _b(dm[1]))
            else:
                ys, yi, yr = (_dot_nt(_b(ub[:, _cols(n)]), _b(dm[n])) for n in range(3 * c - 1, 3 * c + 2))
                ya[:, _cols(2 * c)] = ys - yi
                y = yr - ys if c == 1 else ys - yr
            ya[:, _cols(2 * c + 1)] = y
            return y[0:8]

        def ln_attn(r0, ya, g, gate):
            rr, rows = pl.ds(r0 + 16 * g, 16), pl.ds(16 * g, 16)
            yt = _tiles(ya[rows, :])
            yt[0] = gate(yt[0])
            x0 = X2[rr, :] if last else xin[rr, :].astype(f32)
            xs = [a + b for a, b in zip(_tiles(x0), _radix8_inv(yt))]
            X[rr, :] = jnp.concatenate(xs, axis=1)
            z = jnp.concatenate(_layernorm(xs), axis=1)
            zf[rows, :] = z
            return z

        def operands(get, dst, g, gate):
            top, bot = get(pl.ds(16 * g, 16)), get(pl.ds(H + 16 * g, 16))
            top[0] = gate(top[0])
            for q, a in enumerate(_strassen_lhs(top, bot)):
                w = _w(a)
                dst[q, pl.ds(8 * g, 8), :] = w
            return w

        def strassen(A, B, n, put):
            m = {}

            def mm(q, gate=lambda v: v):
                return _dot(_b(A[q]), _b(gate(B[q, :, _cols(n)])))

            def first(gate):
                m[1], m[2], m[3] = mm(0, gate), mm(1), mm(2)
                c22 = ((m[1] - m[2]) + m[3]) + mm(5)
                put(1, 1, c22)
                return c22[0:8]

            def second(gate):
                m4 = mm(3, gate)
                put(1, 0, m[2] + m4)
                m5 = mm(4)
                put(0, 1, m[3] + m5)
                c11 = ((m[1] + m4) - m5) + mm(6)
                put(0, 0, c11)
                return c11[0:8]
            return [first, second]

        def proj(z, par, n):
            part = n // 4
            dst, t0 = bufs[par][part >> 1], 8 * (part & 1)

            def put(r, c, y):
                dst[t0 + 4 * c + n % 4, pl.ds(16 + r * H, H), :] = y
            return strassen(z, Wq, n, put)

        def softmax(r0, par, rr, gate):
            QK = bufs[par][0]
            q = [QK[j, pl.ds(16 + rr, 8), :] for j in range(8)]
            q[0] = gate(q[0])
            L = []
            for w in range(8):
                p = _tree(jnp.add, [q[j] * QK[8 + j, pl.ds(16 + rr - 2 * w, 8), :] for j in range(8)])
                p = p + pltpu.roll(p, 64, 1)
                p = p + jnp.take_along_axis(p, lane ^ 1, axis=1)
                if rr < 2 * w:
                    p = jnp.where(r0 + rr + sub >= 2 * w, p, -1e9 * 32 ** 0.5)
                L.append(p)
            m = _tree(jnp.maximum, L)
            e = [jnp.exp2((l - m) * float(32 ** -0.5 * np.log2(np.e))) for l in L]
            inv = 1.0 / _tree(jnp.add, e)
            return [v * inv for v in e]

        def mix(par, rr, z8, p):
            VO = bufs[par][1]
            for j in range(8):
                o = _tree(jnp.add, [p[w] * VO[j, pl.ds(16 + rr - 2 * w, 8), :] for w in range(8)])
                VO[8 + j, pl.ds(z8 + rr, 8), :] = o
            return o

        def attend(r0, par, rr, ordered, gate):
            p = softmax(r0, par, rr, gate)
            if ordered:
                QK = bufs[par][0]
                for w in range(8):
                    QK[16 + w, pl.ds(zero8 + rr, 8), :] = p[w]
                p = [QK[16 + w, pl.ds(rr, 8), :] for w in range(8)]
            return mix(par, rr, zero8 if ordered else 0, p)

        def out_proj(r0, ob, yb, n):
            def put(r, c, y):
                at = (pl.ds(r0 + r * H, H), _cols(4 * c + n))
                if last:
                    xin[at] = (X[at] + y).astype(bf16)
                else:
                    yb[pl.ds(r * H, H), _cols(4 * c + n)] = X[at] + y
            return strassen(ob, Wo, n, put)

        def residual(r0, tb, yb, g, gate):
            v = gate(yb[pl.ds(16 * g, 16), :])
            X2[pl.ds(r0 + 16 * g, 16), :] = v
            return ln_radix8(tb, g, _tiles(v))

        def in_pairs(fn):
            def job(cs, gate):
                return [fn(c, gate if c == cs[0] else (lambda v: v)) for c in cs][-1]
            return [P_(job, (0, 1)), P_(job, (2, 3))]
        m_idft = lambda y=ya: in_pairs(P_(idft_d, y))
        v_iop = lambda r0: [P_(idft_operands, r0, c) for c in range(4)]
        m_proj = lambda par, lo=0, hi=12: [j for n in range(lo, hi) for j in proj((z0, z1)[par], par, n)]
        m_out = lambda r0, ob, y=yb: [j for n in range(4) for j in out_proj(r0, ob, y, n)]
        m_dft = lambda r0, tb=tb0: [] if last else in_pairs(P_(dft_d, r0, tb))

        def v_ln(r0, par, y=ya):
            jobs = []
            for g in range(H // 16):
                jobs += [P_(ln_attn, r0, y, g), P_(ln_attn, r0, y, g + H // 16),
                         P_(operands, lambda rows: _tiles(zf[rows, :]), (z0, z1)[par], g)]
            return jobs

        def v_att(r0, par, ordered=True, dst=None):
            jobs = []
            for g in range(H // 16):
                jobs += [P_(attend, r0, par, h + 16 * g + e, ordered) for h in (0, H) for e in (0, 8)]
                jobs += [P_(operands, lambda rows: [bufs[par][1][8 + j, rows, :] for j in range(8)],
                            (o0, o1)[par] if dst is None else dst, g)]
            return jobs
        v_res = lambda r0, tb=tb0, y=yb: [] if last else [P_(residual, r0, tb, y, g) for g in range(T // 16)]

        def halo(par, first=False):
            for j in range(8):
                for dst, src, t in zip(bufs[par], bufs[1 - par], (8 + j, j)):
                    dst[t, 0:16, :] = jnp.zeros((16, 128), f32) if first else src[t, T:T + 16, :]

        def head0():
            halo(0, True)
            weave(m_idft(yb) + m_idft(),
                  _spread(v_iop(0), 0, 0) + _spread(v_iop(T), 2, 2) + _spread(v_ln(0, 0, yb), 2, 4))

        def head(part):
            if part < 2:
                (cp_q[2], cp_o)[part].wait()
            vec = (_spread(gather_jobs(1), 0, 8) + _spread(spin_jobs(2), 0, 8),
                   _spread(gather_jobs(2), 0, 8) + _spread(wo_jobs()[:8], 0, 8),
                   _spread(wo_jobs()[8:], 0, 8))[part]
            weave(m_proj(0, 4 * part, 4 * part + 4), vec + _spread(v_ln(T, 1)[8 * part:8 * part + 8], 0, 8))

        def step(i, par, old=True):
            rn, rp, ro = ((i + d) * T if isinstance(i, int) else pl.multiple_of((i + d) * T, T) for d in (1, -1, -2))
            halo(par)
            mo, mi = m_out(ro, (o0, o1)[par]) if old else [], m_idft()
            a, b = len(mo), len(mo) + len(mi)
            na, nl = (26, 24) if old and not last else (22, 22)
            vec = _spread(v_att(rp, 1 - par), 0, b + na, 4 if old else 3)
            if old:
                vec += _spread(v_res(ro), a, b + 22, 2)
            vec += _spread(v_iop(rn), 0, a, 2 if old else None)
            vec += _spread(v_ln(rn, 1 - par), b, b + nl, 2)
            p, md = m_proj(par), m_dft(ro) if old else []
            weave(mo + mi + p[:22] + md + p[22:], vec)
            if last and old:
                out_copy(ro, i - 2).start()

        r5, r6, r7 = ((NB - d) * T for d in (3, 2, 1))

        def tail0():
            halo(1)
            weave(m_proj(1), _spread(v_att(r6, 0), 0, 22, 4))

        def tail1():
            weave(m_out(r5, o1, ya) + m_out(r6, o0) + m_dft(r5),
                  _spread(v_att(r7, 1, False, z0), 0, 14, 4) + _spread(v_res(r5, tb0, ya), 8, 16, 2))
            if last:
                out_copy(r5, NB - 3).start()
                out_copy(r6, NB - 2).start()

        def tail2():
            weave(m_out(r7, z0, ya) + m_dft(r6), _spread(v_res(r6), 0, 7, 2))
            if last:
                out_copy(r7, NB - 1).start()
            for job in v_res(r7, tb1, ya):
                job(lambda v: v)
            weave(m_dft(r7, tb1), [])

        def head_all():
            weave(m_proj(0), _spread(v_ln(T, 1), 0, 22, 2))
        heads = [head_all] if last else [P_(head, part) for part in range(3)]
        for fn in [head0] + heads + [P_(step, 1, 1, False)]:
            region(fn)

        def loop(i, _):
            for par in range(2):
                pl.when(i % 2 == par)(P_(step, i, par))
            return _
        jax.lax.fori_loop(2, NB - 1, loop, 0)
        for fn in (tail0, tail1, tail2):
            region(fn)

    def run_rowwise(last):
        zs = pltpu.VMEM((7, H // 2, 512), u32)
        rows, qk, vo = pltpu.VMEM((T, D), f32), pltpu.VMEM((24, 16 + T, 128), f32), pltpu.VMEM((16, 16 + T, 128), f32)
        pl.run_scoped(P_(rowwise, last), pltpu.VMEM((T // 2, 11 * 128), u32),
                      rows, rows, rows, zs, zs, zs, zs, qk, qk, vo, vo)

    gen_dm()

    def ln_x(r0, tb, g, gate):
        return ln_radix8(tb, g, _tiles(xin[pl.ds(r0 + 16 * g, 16), :].astype(f32)))

    def first_dft(i, par):
        r0 = pl.multiple_of(i * T, T)
        x_copy(r0, i).wait()

        @pl.when(i + 3 < NB)
        def _():
            x_copy(pl.multiple_of(jnp.minimum(i + 3, NB - 1) * T, T), jnp.minimum(i + 3, NB - 1)).start()

        @pl.when(i + 3 == NB)
        def _():
            for cp in cp_w:
                cp.start()
        weave([P_(dft_d, r0 - T, (tb0, tb1)[1 - par], c) for c in range(4)],
              _spread([P_(ln_x, r0, (tb0, tb1)[par], g) for g in range(T // 16)], 0, 4, 2))

    def first_ln():
        x_copy(0, 0).wait()
        x_copy(3 * T, 3).start()
        weave([], _spread([P_(ln_x, 0, tb0, g) for g in range(T // 16)], 0, 0))

    def first_loop(i, _):
        for par in range(2):
            pl.when(i % 2 == par)(P_(first_dft, i, par))
        return _

    region(first_ln)
    jax.lax.fori_loop(1, NB, first_loop, 0)
    region(lambda: weave([P_(dft_d, (NB - 1) * T, tb1, c) for c in range(4)], _spread(gen_g(False), 0, 4)))
    run_spectral(True)
    run_rowwise(False)
    run_spectral(False)
    run_rowwise(True)
    for i in range(NB):
        out_copy(i * T, i).wait()


@jax.jit
def pallas_interleave_layers__spectral_gfnet__sliding_local_dilated__prompt_kernel(
        A_x, A_w_r, A_w_i, B_x, B_wqkv, B_wo):
    del B_x
    hbm = pl.BlockSpec(memory_space=pltpu.HBM)
    args = (A_x.reshape(S, D), A_w_r.T, A_w_i.T, B_wqkv, B_wo, jnp.asarray(_seeds()))
    out = pl.pallas_call(
        _kernel,
        out_shape=jax.ShapeDtypeStruct((S, D), bf16),
        in_specs=[hbm] * 6,
        out_specs=hbm,
        scratch_shapes=[
            pltpu.VMEM((38, 8, 128), f32),
            pltpu.VMEM((S, D), bf16),
            pltpu.VMEM((S, D), f32),
            pltpu.VMEM((S, D), f32),
            pltpu.VMEM((4, 3, 17 * VPITCH - 1, 128), u32),
            pltpu.VMEM((4, 4, 17 * PITCH - 1, 128), f32),
            pltpu.VMEM((11, 64, 128), u32),
            pltpu.VMEM((16, 3, 64, 128), u32),
            pltpu.VMEM((16, 128, 256), u32),
            pltpu.VMEM((5, S, 128), u32),
            pltpu.VMEM((7, 256, 1536), u32),
            pltpu.VMEM((7, 256, 512), u32),
            pltpu.VMEM((T // 2, 11 * 128), u32),
            pltpu.VMEM((T // 2, 11 * 128), u32),
            pltpu.VMEM((513, S), bf16),
            pltpu.VMEM((513, S), bf16),
            pltpu.VMEM((D, 3 * D), bf16),
            pltpu.VMEM((D, D), bf16),
            pltpu.VMEM((3, 8, 584, 128), u32),
            pltpu.VMEM((16, 520, 128), u32),
            pltpu.SemaphoreType.DMA((NB + 9,)),
        ],
        compiler_params=pltpu.CompilerParams(vmem_limit_bytes=127 * 1024 * 1024),
    )(*args)
    return out.reshape(1, S, D)
```
